```python
import jax
import jax.numpy as jnp

def _softmax(x, axis=-1):
    return jax.nn.softmax(x, axis=axis)

def _gelu(x):
    return jax.nn.gelu(x, approximate=True)

def _silu(x):
    return jax.nn.silu(x)

def _sigmoid(x):
    return jax.nn.sigmoid(x)

def _layernorm(x, axis=-1, eps=1e-05):
    m = jnp.mean(x, axis=axis, keepdims=True)
    v = jnp.var(x, axis=axis, keepdims=True)
    return (x - m) / jnp.sqrt(v + eps)

def _scatter_add(tgt, idx, src, axis=0):
    return tgt.at[idx].add(src)

def _segment_sum(src, seg, n):
    return jax.ops.segment_sum(src, seg, n)

class _Rng:

    def __init__(self, key):
        self._k = key

    def _next(self):
        self._k, sub = jax.random.split(self._k)
        return sub

    def normal(self, shape):
        return jax.random.normal(self._next(), shape, dtype=jnp.bfloat16)

    def randint(self, lo, hi, shape):
        return jax.random.randint(self._next(), shape, lo, hi, dtype=jnp.int32)

    def uniform(self, shape, lo=0.0, hi=1.0):
        return jax.random.uniform(self._next(), shape, jnp.bfloat16, lo, hi)

    def permutation(self, n):
        return jax.random.permutation(self._next(), n)
kernel_name = 'recurrent_scan__ssm_conv_h3__mixer_gmlp__prompt'

def setup_inputs():
    _rng = _Rng(jax.random.key(int.from_bytes(__import__("os").urandom(4), "little")))
    _w = lambda a: (lambda t: t.astype(jnp.bfloat16) if jnp.issubdtype(t.dtype, jnp.floating) else t)(jnp.asarray(a))

    def _A_setup():
        B, S, D = (1, 2048, 640)
        ks = 4
        return {'q': _w((lambda *s: _rng.normal(s) * 0.05)(B, S, D)), 'k': _w((lambda *s: _rng.normal(s) * 0.05)(B, S, D)), 'v': _w((lambda *s: _rng.normal(s) * 0.05)(B, S, D)), 'shift_k': _w((lambda *s: _rng.normal(s) * 0.05)(D, ks) * 0.5), 'ssm_k': _w((lambda *s: _rng.normal(s) * 0.05)(D, S) * (1.0 / S ** 0.5)), 'ssm_D': _w((lambda *s: _rng.normal(s) * 0.05)(D))}
    _A_in = _A_setup()

    def _B_setup():
        B, S, D, F = (1, 2048, 640, 1536)
        Fh = F // 2
        return {'x': _w((lambda *s: _rng.normal(s) * 0.05)(B, S, D)), 'w_in': _w((lambda *s: _rng.normal(s) * 0.05)(D, 2 * Fh)), 'w_sp': _w(0.01 * (lambda *s: _rng.normal(s) * 0.05)(S, S)), 'b_sp': _w(1.0 + 0.01 * (lambda *s: _rng.normal(s) * 0.05)(S)), 'w_out': _w((lambda *s: _rng.normal(s) * 0.05)(Fh, D))}
    _B_in = _B_setup()
    return {'A_q': _A_in['q'], 'A_k': _A_in['k'], 'A_v': _A_in['v'], 'A_shift_k': _A_in['shift_k'], 'A_ssm_k': _A_in['ssm_k'], 'A_ssm_D': _A_in['ssm_D'], 'B_x': _B_in['x'], 'B_w_in': _B_in['w_in'], 'B_w_sp': _B_in['w_sp'], 'B_b_sp': _B_in['b_sp'], 'B_w_out': _B_in['w_out']}

def reference(A_q, A_k, A_v, A_shift_k, A_ssm_k, A_ssm_D, B_x, B_w_in, B_w_sp, B_b_sp, B_w_out):

    def _A_ref(q, k, v, shift_k, ssm_k, ssm_D):
        B, S, D = q.shape
        ks = shift_k.shape[-1]
        k_pad = jnp.pad(k, ((0, 0), (ks - 1, 0), (0, 0)))
        k_shift = jnp.zeros_like(k)
        for t in range(ks):
            k_shift = k_shift + k_pad[:, t:t + S, :] * shift_k[:, ks - 1 - t][None, None, :]
        kv = k_shift * v
        L = 2 * S
        kv_pad = jnp.pad(kv, ((0, 0), (0, S), (0, 0)))
        kf_pad = jnp.pad(ssm_k, ((0, 0), (0, S)))
        kv_f = (lambda x, axes=(-2, -1): jnp.fft.rfft2(x.astype(jnp.float32), axes=axes))(kv_pad[:, None, :, :], axes=(1, 2))
        kf_f = (lambda x, axes=(-2, -1): jnp.fft.rfft2(x.astype(jnp.float32), axes=axes))(kf_pad[:, None, :], axes=(1, 2))
        kf_f = (lambda x, *d: x.transpose(*d))(kf_f, 1, 2, 0)
        y_f = kv_f * kf_f[None, :, :, :]
        y = (lambda x, s, axes=(-2, -1): jnp.fft.irfft2(x, s=s, axes=axes).astype(jnp.bfloat16))(y_f, (1, L), axes=(1, 2))[:, 0, :S, :]
        y = y + kv * ssm_D[None, None, :]
        return q * y

    def _B_ref(x, w_in, w_sp, b_sp, w_out):
        B, S, D = x.shape
        F = w_in.shape[-1]
        Fh = F // 2
        z = _gelu(jnp.einsum('bsd,df->bsf', x, w_in))
        z1 = z[..., :Fh].copy()
        z2 = _layernorm(z[..., Fh:], axis=-1)
        g = jnp.einsum('ts,bsf->btf', w_sp, z2) + b_sp[None, :, None]
        return jnp.einsum('bsf,fd->bsd', z1 * g, w_out)
    x = A_q
    xn = _layernorm(x, axis=-1)
    s = _A_ref(xn, A_k, A_v, A_shift_k, A_ssm_k, A_ssm_D)
    g = _silu(_B_ref(xn, B_w_in, B_w_sp, B_b_sp, B_w_out))
    return x + s * g
```

```python
import numpy as np
import jax
import jax.numpy as jnp
import jax.experimental.pallas as pl
import jax.experimental.pallas.tpu as pltpu

_C = 128


def _dft_mats():
    n = np.arange(_C)
    f = np.concatenate([np.arange(0, _C, 2), np.arange(1, _C, 2)])
    th = 2.0 * np.pi * (f[:, None] + 0.5) * n[None, :] / (2 * _C)
    fwd = np.concatenate([np.cos(th), -np.sin(th)], axis=0)
    inv = np.concatenate([np.cos(th).T, -np.sin(th).T], axis=1) / _C
    return fwd.astype(np.float32), inv.astype(np.float32)


_FWD, _INV = _dft_mats()


def _ln(x):
    m = jnp.mean(x, axis=-1, keepdims=True)
    xc = x - m
    v = jnp.mean(xc * xc, axis=-1, keepdims=True)
    return xc * jax.lax.rsqrt(v + 1e-5)


def pallas_recurrent_scan__ssm_conv_h3__mixer_gmlp__prompt_kernel(
    A_q: jax.Array,
    A_k: jax.Array,
    A_v: jax.Array,
    A_shift_k: jax.Array,
    A_ssm_k: jax.Array,
    A_ssm_D: jax.Array,
    B_x: jax.Array,
    B_w_in: jax.Array,
    B_w_sp: jax.Array,
    B_b_sp: jax.Array,
    B_w_out: jax.Array,
):
    del B_x
    _, S, D = A_q.shape
    KS = A_shift_k.shape[-1]
    F2 = B_w_in.shape[-1]
    FH = F2 // 2
    T = 512
    NT = S // T
    CPT = T // _C
    NC = S // _C
    FB = _C // NT
    HALO = 8
    bf16, f32 = jnp.bfloat16, jnp.float32

    def kernel(q_h, k_h, v_h, ssm_h, win_h, wsp_h, wout_h,
               shift_ref, dvec_ref, bsp_ref, fwd_ref, inv_ref,
               o_ref,
               q_v, k_v, v_v, ssm_v, win_v, wsp_v, wout_v,
               xn_s, kv_s, z1_s, z2_s, xf_s, kf_s, sf_s, kpad_s, shift_s,
               sems):
        step = pl.program_id(0)

        def rows(t):
            return pl.ds(pl.multiple_of(t * T, T), T)

        def tile_copies(t):
            r = rows(t)
            return (
                pltpu.make_async_copy(q_h.at[0, r, :], q_v.at[r, :], sems.at[0, t]),
                pltpu.make_async_copy(k_h.at[0, r, :], k_v.at[r, :], sems.at[1, t]),
                pltpu.make_async_copy(v_h.at[0, r, :], v_v.at[r, :], sems.at[2, t]),
                pltpu.make_async_copy(ssm_h.at[:, r], ssm_v.at[:, r], sems.at[3, t]),
            )

        def wsp_copy(t):
            r = rows(t)
            return pltpu.make_async_copy(wsp_h.at[r, :], wsp_v.at[r, :], sems.at[4, t])

        def win_copy():
            return pltpu.make_async_copy(win_h, win_v, sems.at[5, 0])

        def wout_copy():
            return pltpu.make_async_copy(wout_h, wout_v, sems.at[5, 1])

        @pl.when(step == 0)
        def _():
            cq, ck, cv, cs = tile_copies(0)
            cq.start()
            win_copy().start()
            ck.start()
            cv.start()
            cs.start()
            kpad_s[0:HALO, :] = jnp.zeros((HALO, D), f32)
            sk = shift_ref[...].astype(f32)
            eye = (jax.lax.broadcasted_iota(jnp.int32, (8, KS), 0)
                   == jax.lax.broadcasted_iota(jnp.int32, (8, KS), 1)).astype(bf16)
            shift_s[...] = jax.lax.dot_general(
                eye, shift_ref[...], (((1,), (1,)), ((), ())),
                preferred_element_type=f32)

        @pl.when(step < NT)
        def _():
            t = step

            @pl.when(t + 1 < NT)
            def _():
                for c in tile_copies(t + 1):
                    c.start()

            wsp_copy(t).start()

            @pl.when(t == 1)
            def _():
                wout_copy().start()

            cq, ck, cv, cs = tile_copies(t)
            r = rows(t)
            cq.wait()
            xn = _ln(q_v[r, :].astype(f32)).astype(bf16)
            xn_s[r, :] = xn

            @pl.when(t == 0)
            def _():
                win_copy().wait()

            z = jnp.dot(xn, win_v[...], preferred_element_type=f32)
            z = jax.nn.gelu(z, approximate=True)
            z1_s[r, :] = z[:, :FH].astype(bf16)
            z2_s[r, :] = _ln(z[:, FH:]).astype(bf16)

            ck.wait()
            cv.wait()
            kpad_s[HALO:HALO + T, :] = k_v[r, :].astype(f32)
            ksh = kpad_s[HALO:HALO + T, :] * shift_s[0:1, :]
            for j in range(1, KS):
                ksh = ksh + kpad_s[HALO - j:HALO - j + T, :] * shift_s[j:j + 1, :]
            kpad_s[0:HALO, :] = kpad_s[T:T + HALO, :]
            kv = (ksh * v_v[r, :].astype(f32)).astype(bf16)
            kv_s[r, :] = kv
            fwd = fwd_ref[...]
            cs.wait()
            for c in range(CPT):
                xf_s[t * CPT + c] = jnp.dot(fwd, kv[c * _C:(c + 1) * _C, :],
                                            preferred_element_type=f32)
                blk = ssm_v[:, pl.ds(pl.multiple_of(t * T + c * _C, _C), _C)]
                kf_s[t * CPT + c] = jax.lax.dot_general(
                    fwd, blk, (((1,), (1,)), ((), ())), preferred_element_type=f32)

        @pl.when(jnp.logical_and(step >= NT, step < 2 * NT))
        def _():
            t = step - NT
            r = rows(t)
            wsp_copy(t).wait()
            g = jnp.dot(wsp_v[r, :], z2_s[...], preferred_element_type=f32)
            b = bsp_ref[:, r].astype(f32)
            bcol = jnp.transpose(jnp.broadcast_to(b, (128, T)))
            for c in range(FH // 128):
                cs_ = slice(c * 128, (c + 1) * 128)
                h = z1_s[r, cs_].astype(f32) * (g[:, cs_] + bcol)
                z1_s[r, cs_] = h.astype(bf16)

            for fb in range(FB // 8):
                f0 = pl.multiple_of(t * FB + fb * 8, 8)
                fre = pl.ds(f0, 8)
                fim = pl.ds(f0 + _C, 8)
                for i in range(NC):
                    are = aim = None
                    for j in range(i + 1):
                        xr = xf_s[j, fre, :]
                        xi = xf_s[j, fim, :]
                        kr = kf_s[i - j, fre, :]
                        ki = kf_s[i - j, fim, :]
                        if are is None:
                            are = xr * kr - xi * ki
                            aim = xr * ki + xi * kr
                        else:
                            are = are + xr * kr - xi * ki
                            aim = aim + xr * ki + xi * kr
                    sf_s[i, fre, :] = are
                    sf_s[i, fim, :] = aim

        @pl.when(step >= 2 * NT)
        def _():
            t = step - 2 * NT
            r = rows(t)

            @pl.when(t == 0)
            def _():
                wout_copy().wait()

            o = jnp.dot(z1_s[r, :], wout_v[...], preferred_element_type=f32)
            gate = o * jax.nn.sigmoid(o)
            inv = inv_ref[...]
            H = _C // 2
            for c in range(CPT):
                i = t * CPT + c
                cur = sf_s[i]
                prv = sf_s[jnp.maximum(i - 1, 0)]
                if c == 0:
                    prv = jnp.where(t > 0, prv, 0.0)
                pre, pim = prv[:_C], prv[_C:]
                add = jnp.concatenate(
                    [-pim[:H], pim[H:], pre[:H], -pre[H:]], axis=0)
                tt = (cur + add).astype(bf16)
                y = jnp.dot(inv, tt, preferred_element_type=f32)
                rc = pl.ds(pl.multiple_of(t * T + c * _C, _C), _C)
                y = y + kv_s[rc, :].astype(f32) * dvec_ref[...].astype(f32)
                s = xn_s[rc, :].astype(f32) * y
                out = q_v[rc, :].astype(f32) + s * gate[c * _C:(c + 1) * _C, :]
                o_ref[c * _C:(c + 1) * _C, :] = out.astype(o_ref.dtype)

    full = lambda shape: pl.BlockSpec(shape, lambda s: (0,) * len(shape))
    anyspec = pl.BlockSpec(memory_space=pl.ANY)
    out = pl.pallas_call(
        kernel,
        grid=(3 * NT,),
        in_specs=[anyspec] * 7 + [
            full((D, KS)), full((1, D)), full((1, S)),
            full((2 * _C, _C)), full((_C, 2 * _C)),
        ],
        out_specs=pl.BlockSpec((None, T, D),
                               lambda s: (0, jnp.maximum(s - 2 * NT, 0), 0)),
        out_shape=jax.ShapeDtypeStruct((1, S, D), A_q.dtype),
        scratch_shapes=[
            pltpu.VMEM((S, D), bf16), pltpu.VMEM((S, D), bf16),
            pltpu.VMEM((S, D), bf16), pltpu.VMEM((D, S), bf16),
            pltpu.VMEM((D, F2), bf16), pltpu.VMEM((S, S), bf16),
            pltpu.VMEM((FH, D), bf16),
            pltpu.VMEM((S, D), bf16), pltpu.VMEM((S, D), bf16),
            pltpu.VMEM((S, FH), bf16), pltpu.VMEM((S, FH), bf16),
            pltpu.VMEM((NC, 2 * _C, D), f32), pltpu.VMEM((NC, 2 * _C, D), f32),
            pltpu.VMEM((NC, 2 * _C, D), f32),
            pltpu.VMEM((T + HALO, D), f32), pltpu.VMEM((8, D), f32),
            pltpu.SemaphoreType.DMA((6, NT)),
        ],
        compiler_params=pltpu.CompilerParams(
            dimension_semantics=("arbitrary",),
            vmem_limit_bytes=110 * 1024 * 1024,
        ),
    )(A_q, A_k, A_v, A_ssm_k, B_w_in, B_w_sp, B_w_out,
      A_shift_k, A_ssm_D.reshape(1, D), B_b_sp.reshape(1, S),
      jnp.asarray(_FWD, bf16), jnp.asarray(_INV, bf16))
    return out
```

```python
import numpy as np
import jax
import jax.numpy as jnp
import jax.experimental.pallas as pl
import jax.experimental.pallas.tpu as pltpu

_C = 128


def _dft_mats():
    n = np.arange(_C)
    f = np.concatenate([np.arange(0, _C, 2), np.arange(1, _C, 2)])
    th = 2.0 * np.pi * (f[:, None] + 0.5) * n[None, :] / (2 * _C)
    fwd = np.concatenate([np.cos(th), -np.sin(th)], axis=0)
    inv = np.concatenate([np.cos(th).T, -np.sin(th).T], axis=1) / _C
    return fwd.astype(np.float32), inv.astype(np.float32)


_FWD, _INV = _dft_mats()
_OPT = dict(RB=32, LB=16, MB=512, order=[
    ("K", 0), ("K", 1), ("K", 2), ("K", 3), ("P", 0), ("P", 1), ("P", 2), ("P", 3),
    ("Z", 1024, 1536), ("V", 0), ("X", 0), ("V", 1), ("X", 1), "lnx",
    ("Z", 512, 1024), ("V", 2), ("X", 2), ("V", 3), ("X", 3), "halo",
    ("Z", 0, 512), "lnz"],
    order0=["q0", "ln0", "w2", ("Z", 1024, 1536), "ssm", ("K", 0), ("K", 1), ("K", 2), ("K", 3),
            "w1", ("Z", 512, 1024), "kv", ("P", 0), ("P", 1), ("P", 2), ("P", 3), "prefetch",
            ("V", 0), ("X", 0), ("V", 1), ("X", 1), ("V", 2), ("X", 2), ("V", 3), ("X", 3), "halo",
            "w0", "q1", ("Z", 0, 512), "lnz", "lnx"])


def _ln(x):
    m = jnp.mean(x, axis=-1, keepdims=True)
    xc = x - m
    v = jnp.mean(xc * xc, axis=-1, keepdims=True)
    return xc * jax.lax.rsqrt(v + 1e-5)


def pallas_recurrent_scan__ssm_conv_h3__mixer_gmlp__prompt_kernel(
    A_q: jax.Array,
    A_k: jax.Array,
    A_v: jax.Array,
    A_shift_k: jax.Array,
    A_ssm_k: jax.Array,
    A_ssm_D: jax.Array,
    B_x: jax.Array,
    B_w_in: jax.Array,
    B_w_sp: jax.Array,
    B_b_sp: jax.Array,
    B_w_out: jax.Array,
):
    del B_x
    _, S, D = A_q.shape
    KS = A_shift_k.shape[-1]
    F2 = B_w_in.shape[-1]
    FH = F2 // 2
    T = 512
    NT = S // T
    CPT = T // _C
    NC = S // _C
    FB = _C // NT
    HALO = 8
    NW_COLS = 128
    bf16, f32 = jnp.bfloat16, jnp.float32

    def kernel(q_h, k_h, v_h, ssm_h, win_h, wsp_h, wout_h,
               shift_ref, dvec_ref, bsp_ref, fwd_ref, inv_ref,
               o_ref,
               q_v, k_v, v_v, ssm_v, win_v, wsp_v, wout_v,
               xn_s, kv_s, z1_s, z2_s, xf_s, kf_s, sf_s, kpad_s, shift_s, z2f_s, xn2_s, zero_s,
               sems):
        step = pl.program_id(0)

        def rows(t):
            return pl.ds(pl.multiple_of(t * T, T), T)

        def q_copy(t):
            r = rows(t)
            return pltpu.make_async_copy(q_h.at[0, r, :], q_v.at[r, :], sems.at[0, t])

        def tile_copies(t):
            r = rows(t)
            return (
                pltpu.make_async_copy(k_h.at[0, r, :], k_v.at[r, :], sems.at[1, t]),
                pltpu.make_async_copy(v_h.at[0, r, :], v_v.at[r, :], sems.at[2, t]),
                pltpu.make_async_copy(ssm_h.at[:, r], ssm_v.at[:, r], sems.at[3, t]),
            )

        def wsp_copy(t):
            r = rows(t)
            return pltpu.make_async_copy(wsp_h.at[r, :], wsp_v.at[r, :], sems.at[4, t])

        def win_copy(c):
            cs_ = pl.ds(c * 512, 512)
            return pltpu.make_async_copy(win_h.at[:, cs_], win_v.at[:, cs_], sems.at[6, c])

        def wout_copy():
            return pltpu.make_async_copy(wout_h, wout_v, sems.at[5, 1])

        @pl.when(step == 0)
        def _():
            ck, cv, cs = tile_copies(0)
            q_copy(0).start()
            win_copy(2).start()
            cs.start()
            win_copy(1).start()
            ck.start()
            cv.start()
            win_copy(0).start()
            q_copy(1).start()
            kpad_s[0:HALO, :] = jnp.zeros((HALO, D), f32)
            zero_s[0] = 0
            shift_s[0:KS, :] = shift_ref[...].astype(f32)

        @pl.when(step < NT)
        @jax.named_scope('phB')
        def _():
            t = step

            tn = jnp.minimum(t + 1, NT - 1)

            def prefetch():
                @pl.when(t + 1 < NT)
                def _():
                    for c in tile_copies(t + 1):
                        c.start()

                @pl.when(t + 2 < NT)
                def _():
                    q_copy(t + 2).start()

                wsp_copy(t).start()

                @pl.when(t == 1)
                def _():
                    wout_copy().start()

            r = rows(t)
            ck, cv, cs = tile_copies(t)

            def ln0():
                for c in range(T // 16):
                    rc = slice(c * 16, (c + 1) * 16)
                    xn_s[rc, :] = _ln(q_v[rc, :].astype(f32)).astype(bf16)

            fwd = fwd_ref[...]
            O = _OPT

            def kdft(c):
                blk = ssm_v[:, pl.ds(pl.multiple_of(t * T + c * _C, _C), _C)]
                kf_s[t * CPT + c] = jax.lax.dot_general(
                    fwd, blk, (((1,), (1,)), ((), ())), preferred_element_type=f32)

            def gelu(z):
                return jax.nn.gelu(z, approximate=True)

            RB = O["RB"]

            def kpad(c):
                rc = pl.ds(pl.multiple_of(t * T + c * _C, _C), _C)
                kpad_s[HALO + c * _C:HALO + (c + 1) * _C, :] = k_v[rc, :].astype(f32)

            def kv_chunk(c):
                for u in range(_C // RB):
                    o = HALO + c * _C + u * RB
                    ksh = kpad_s[o:o + RB, :] * shift_s[0:1, :]
                    for j in range(1, KS):
                        ksh = ksh + kpad_s[o - j:o - j + RB, :] * shift_s[j:j + 1, :]
                    rc = pl.ds(pl.multiple_of(t * T + c * _C + u * RB, RB), RB)
                    kv_s[rc, :] = (ksh * v_v[rc, :].astype(f32)).astype(bf16)

            def xdft(c):
                rc = pl.ds(pl.multiple_of(t * T + c * _C, _C), _C)
                xf_s[t * CPT + c] = jnp.dot(fwd, kv_s[rc, :], preferred_element_type=f32)

            def lnx():
                LB = O["LB"]
                for u in range(T // LB):
                    rc = pl.ds(pl.multiple_of(tn * T + u * LB, LB), LB)
                    xn2_s[u * LB:(u + 1) * LB, :] = _ln(q_v[rc, :].astype(f32)).astype(bf16)

            def lnz():
                LB = O["LB"]
                for u in range(T // LB):
                    rc = pl.ds(pl.multiple_of(t * T + u * LB, LB), LB)
                    z2_s[rc, :] = _ln(z2f_s[u * LB:(u + 1) * LB, :]).astype(bf16)

            def zdot(c0, c1):
                MB = O["MB"]
                for m in range(T // MB):
                    rm = pl.ds(pl.multiple_of(t * T + m * MB, MB), MB)
                    z = jnp.dot(xn_s[rm, :], win_v[:, c0:c1], preferred_element_type=f32)
                    for cc in range(c0, c1, 128):
                        gz = gelu(z[:, cc - c0:cc - c0 + 128])
                        if cc >= FH:
                            z2f_s[m * MB:(m + 1) * MB, cc - FH:cc - FH + 128] = gz
                        else:
                            z1_s[rm, cc:cc + 128] = gz.astype(bf16)

            def halo():
                kpad_s[0:HALO, :] = kpad_s[T:T + HALO, :]

            fns = dict(K=kdft, P=kpad, V=kv_chunk, X=xdft, Z=zdot)
            waits = dict(q0=lambda: q_copy(0).wait(), ssm=cs.wait,
                         kv=lambda: (ck.wait(), cv.wait()),
                         q1=lambda: q_copy(tn).wait(),
                         w0=lambda: win_copy(0).wait(), w1=lambda: win_copy(1).wait(),
                         w2=lambda: win_copy(2).wait())

            def body(order):
                for item in order:
                    if item == "lnx":
                        lnx()
                    elif item == "lnz":
                        lnz()
                    elif item == "halo":
                        halo()
                    elif item == "ln0":
                        ln0()
                    elif item == "prefetch":
                        prefetch()
                    elif item in waits:
                        waits[item]()
                    else:
                        fns[item[0]](*item[1:])
                xn_s[rows(tn), :] = xn2_s[...]

            @pl.when(t == 0)
            def _():
                body(O["order0"])

            @pl.when(t > 0)
            def _():
                prefetch()
                cs.wait()
                ck.wait()
                cv.wait()

                @pl.when(t + 1 < NT)
                def _():
                    q_copy(t + 1).wait()

                body(O["order"])

        @pl.when(jnp.logical_and(step >= NT, step < 2 * NT))
        @jax.named_scope('phC1')
        def _():
            t = step - NT
            r = rows(t)
            wsp_copy(t).wait()
            b = bsp_ref[r].astype(f32).reshape(1, T)
            bcol = jnp.transpose(jnp.broadcast_to(b, (128, T)))

            def mac(fb, lt, outs):
                f0 = pl.multiple_of(t * FB + fb * 8, 8)
                fre = pl.ds(f0, 8)
                fim = pl.ds(f0 + _C, 8)
                ls = slice(lt * 128, (lt + 1) * 128)
                for i in outs:
                    are = aim = None
                    for j in range(i + 1):
                        xr = xf_s[j, fre, ls]
                        xi = xf_s[j, fim, ls]
                        kr = kf_s[i - j, fre, ls]
                        ki = kf_s[i - j, fim, ls]
                        if are is None:
                            are = xr * kr - xi * ki
                            aim = xr * ki + xi * kr
                        else:
                            are = are + xr * kr - xi * ki
                            aim = aim + xr * ki + xi * kr
                    sf_s[i, fre, ls] = are
                    sf_s[i, fim, ls] = aim

            groups = [[i, NC - 1 - i] for i in range(NC // 2)]
            work = [(fb, lt, g_) for fb in range(FB // 8) for lt in range(D // 128) for g_ in groups]
            pace = pl.ds(pl.multiple_of(zero_s[0] * 8, 8), 8)
            KQ = 4
            nround = (FH // 128) * KQ
            wi = 0
            for c in range(FH // 128):
                cs_ = slice(c * 128, (c + 1) * 128)
                acc = None
                for kq in range(KQ):
                    ks_ = slice(kq * (S // KQ), (kq + 1) * (S // KQ))
                    p = jnp.dot(wsp_v[r, ks_], z2_s[ks_, cs_], preferred_element_type=f32)
                    acc = p if acc is None else acc + p
                    rd = c * KQ + kq
                    hi = -(-len(work) * (rd + 1) // nround)
                    n = hi - wi
                    for q_, w in enumerate(work[wi:hi]):
                        row = (q_ * T // n) // 8 * 8
                        xf_s[NC, pace, 0:128] = p[row:row + 8, :]
                        mac(*w)
                    wi = hi
                h = z1_s[r, cs_].astype(f32) * (acc + bcol)
                z1_s[r, cs_] = h.astype(bf16)

        @pl.when(step >= 2 * NT)
        @jax.named_scope('phC2')
        def _():
            t = step - 2 * NT
            r = rows(t)

            @pl.when(t == 0)
            def _():
                wout_copy().wait()

            o = jnp.dot(z1_s[r, :], wout_v[...], preferred_element_type=f32)
            gate = o * jax.nn.sigmoid(o)
            inv = inv_ref[...]
            dvec = dvec_ref[...].astype(f32).reshape(1, D)
            H = _C // 2
            for c in range(CPT):
                i = t * CPT + c
                cur = sf_s[i]
                prv = sf_s[jnp.maximum(i - 1, 0)]
                if c == 0:
                    prv = jnp.where(t > 0, prv, 0.0)
                pre, pim = prv[:_C], prv[_C:]
                add = jnp.concatenate(
                    [-pim[:H], pim[H:], pre[:H], -pre[H:]], axis=0)
                tt = (cur + add).astype(bf16)
                y = jnp.dot(inv, tt, preferred_element_type=f32)
                rc = pl.ds(pl.multiple_of(t * T + c * _C, _C), _C)
                y = y + kv_s[rc, :].astype(f32) * dvec
                s = xn_s[rc, :].astype(f32) * y
                out = q_v[rc, :].astype(f32) + s * gate[c * _C:(c + 1) * _C, :]
                o_ref[c * _C:(c + 1) * _C, :] = out.astype(o_ref.dtype)

    full = lambda shape: pl.BlockSpec(shape, lambda s: (0,) * len(shape))
    anyspec = pl.BlockSpec(memory_space=pl.ANY)
    out = pl.pallas_call(
        kernel,
        grid=(3 * NT,),
        in_specs=[anyspec] * 7 + [
            full((KS, D)), full((D,)), full((S,)),
            full((2 * _C, _C)), full((_C, 2 * _C)),
        ],
        out_specs=pl.BlockSpec((None, T, D),
                               lambda s: (0, jnp.maximum(s - 2 * NT, 0), 0)),
        out_shape=jax.ShapeDtypeStruct((1, S, D), A_q.dtype),
        scratch_shapes=[
            pltpu.VMEM((S + 32, D), bf16), pltpu.VMEM((S, D), bf16),
            pltpu.VMEM((S, D), bf16), pltpu.VMEM((D, S), bf16),
            pltpu.VMEM((D, F2), bf16), pltpu.VMEM((S, S), bf16),
            pltpu.VMEM((FH, D), bf16),
            pltpu.VMEM((S, D), bf16), pltpu.VMEM((S, D), bf16),
            pltpu.VMEM((S, FH), bf16), pltpu.VMEM((S, FH), bf16),
            pltpu.VMEM((NC + 1, 2 * _C, D), f32), pltpu.VMEM((NC, 2 * _C, D), f32),
            pltpu.VMEM((NC, 2 * _C, D), f32),
            pltpu.VMEM((T + HALO + 16, D), f32), pltpu.VMEM((8, D), f32),
            pltpu.VMEM((T + 16, FH), f32), pltpu.VMEM((T, D), bf16),
            pltpu.SMEM((1,), jnp.int32),
            pltpu.SemaphoreType.DMA((7, NT)),
        ],
        compiler_params=pltpu.CompilerParams(
            dimension_semantics=("arbitrary",),
            vmem_limit_bytes=110 * 1024 * 1024,
        ),
    )(A_q, A_k, A_v, A_ssm_k, B_w_in, B_w_sp, B_w_out,
      A_shift_k.T, A_ssm_D, B_b_sp,
      jnp.asarray(_FWD, bf16), jnp.asarray(_INV, bf16))
    return out
```

```python
import numpy as np
import jax
import jax.numpy as jnp
import jax.experimental.pallas as pl
import jax.experimental.pallas.tpu as pltpu

_C = 128


def _dft_mats():
    n = np.arange(_C)
    f = np.concatenate([np.arange(0, _C, 2), np.arange(1, _C, 2)])
    th = 2.0 * np.pi * (f[:, None] + 0.5) * n[None, :] / (2 * _C)
    fwd = np.concatenate([np.cos(th), -np.sin(th)], axis=0)
    inv = np.concatenate([np.cos(th).T, -np.sin(th).T], axis=1) / _C
    return fwd.astype(np.float32), inv.astype(np.float32)


_FWD, _INV = _dft_mats()
_OPT = dict(late_gelu=False, KQ=4, groups=[[i] for i in range(16)], RB=32, LB=16, MB=512, order=[
    ("K", 0), ("K", 1), ("K", 2), ("K", 3), ("P", 0), ("P", 1), ("P", 2), ("P", 3),
    ("Z", 1024, 1536), ("V", 0), ("X", 0), ("V", 1), ("X", 1), "lnx",
    ("Z", 512, 1024), ("V", 2), ("X", 2), ("V", 3), ("X", 3), "halo",
    ("Z", 0, 512), "lnz"],
    order0=["q0", "ln0", "w2", ("Z", 1024, 1536), "ssm", ("K", 0), ("K", 1), ("K", 2), ("K", 3),
            "w1", ("Z", 512, 1024), "kv", ("P", 0), ("P", 1), ("P", 2), ("P", 3), "prefetch",
            ("V", 0), ("X", 0), ("V", 1), ("X", 1), ("V", 2), ("X", 2), ("V", 3), ("X", 3), "halo",
            "w0", "q1", ("Z", 0, 512), "lnz", "lnx"])


def _ln(x):
    m = jnp.mean(x, axis=-1, keepdims=True)
    xc = x - m
    v = jnp.mean(xc * xc, axis=-1, keepdims=True)
    return xc * jax.lax.rsqrt(v + 1e-5)


def pallas_recurrent_scan__ssm_conv_h3__mixer_gmlp__prompt_kernel(
    A_q: jax.Array,
    A_k: jax.Array,
    A_v: jax.Array,
    A_shift_k: jax.Array,
    A_ssm_k: jax.Array,
    A_ssm_D: jax.Array,
    B_x: jax.Array,
    B_w_in: jax.Array,
    B_w_sp: jax.Array,
    B_b_sp: jax.Array,
    B_w_out: jax.Array,
):
    del B_x
    _, S, D = A_q.shape
    KS = A_shift_k.shape[-1]
    F2 = B_w_in.shape[-1]
    FH = F2 // 2
    T = 512
    NT = S // T
    CPT = T // _C
    NC = S // _C
    FB = _C // NT
    HALO = 8
    NW_COLS = 128
    bf16, f32 = jnp.bfloat16, jnp.float32

    def kernel(q_h, k_h, v_h, ssm_h, win_h, wsp_h, wout_h,
               shift_ref, dvec_ref, bsp_ref, fwd_ref, inv_ref,
               o_ref,
               q_v, k_v, v_v, ssm_v, win_v, wsp_v, wout_v,
               xn_s, kv_s, z1_s, z2_s, xf_s, kf_s, sf_s, kpad_s, shift_s, z2f_s, xn2_s, zero_s,
               sems):
        step = pl.program_id(0)

        def rows(t):
            return pl.ds(pl.multiple_of(t * T, T), T)

        def q_copy(t):
            r = rows(t)
            return pltpu.make_async_copy(q_h.at[0, r, :], q_v.at[r, :], sems.at[0, t])

        def tile_copies(t):
            r = rows(t)
            return (
                pltpu.make_async_copy(k_h.at[0, r, :], k_v.at[r, :], sems.at[1, t]),
                pltpu.make_async_copy(v_h.at[0, r, :], v_v.at[r, :], sems.at[2, t]),
                pltpu.make_async_copy(ssm_h.at[:, r], ssm_v.at[:, r], sems.at[3, t]),
            )

        def wsp_copy(t):
            r = rows(t)
            return pltpu.make_async_copy(wsp_h.at[r, :], wsp_v.at[r, :], sems.at[4, t])

        def win_copy(c):
            cs_ = pl.ds(c * 512, 512)
            return pltpu.make_async_copy(win_h.at[:, cs_], win_v.at[:, cs_], sems.at[6, c])

        def wout_copy():
            return pltpu.make_async_copy(wout_h, wout_v, sems.at[5, 1])

        @pl.when(step == 0)
        def _():
            ck, cv, cs = tile_copies(0)
            q_copy(0).start()
            win_copy(2).start()
            cs.start()
            win_copy(1).start()
            ck.start()
            cv.start()
            win_copy(0).start()
            q_copy(1).start()
            kpad_s[0:HALO, :] = jnp.zeros((HALO, D), f32)
            zero_s[0] = 0
            shift_s[0:KS, :] = shift_ref[...].astype(f32)

        @pl.when(step < NT)
        @jax.named_scope('phB')
        def _():
            t = step

            tn = jnp.minimum(t + 1, NT - 1)

            def prefetch():
                @pl.when(t + 1 < NT)
                def _():
                    for c in tile_copies(t + 1):
                        c.start()

                @pl.when(t + 2 < NT)
                def _():
                    q_copy(t + 2).start()

                wsp_copy(t).start()

                @pl.when(t == 1)
                def _():
                    wout_copy().start()

            r = rows(t)
            ck, cv, cs = tile_copies(t)

            def ln0():
                for c in range(T // 16):
                    rc = slice(c * 16, (c + 1) * 16)
                    xn_s[rc, :] = _ln(q_v[rc, :].astype(f32)).astype(bf16)

            fwd = fwd_ref[...]
            O = _OPT

            def kdft(c):
                blk = ssm_v[:, pl.ds(pl.multiple_of(t * T + c * _C, _C), _C)]
                kf_s[t * CPT + c] = jax.lax.dot_general(
                    fwd, blk, (((1,), (1,)), ((), ())), preferred_element_type=f32)

            def gelu(z):
                return jax.nn.gelu(z, approximate=True)

            RB = O["RB"]

            def kpad(c):
                rc = pl.ds(pl.multiple_of(t * T + c * _C, _C), _C)
                kpad_s[HALO + c * _C:HALO + (c + 1) * _C, :] = k_v[rc, :].astype(f32)

            def kv_chunk(c):
                for u in range(_C // RB):
                    o = HALO + c * _C + u * RB
                    ksh = kpad_s[o:o + RB, :] * shift_s[0:1, :]
                    for j in range(1, KS):
                        ksh = ksh + kpad_s[o - j:o - j + RB, :] * shift_s[j:j + 1, :]
                    rc = pl.ds(pl.multiple_of(t * T + c * _C + u * RB, RB), RB)
                    kv_s[rc, :] = (ksh * v_v[rc, :].astype(f32)).astype(bf16)

            def xdft(c):
                rc = pl.ds(pl.multiple_of(t * T + c * _C, _C), _C)
                xf_s[t * CPT + c] = jnp.dot(fwd, kv_s[rc, :], preferred_element_type=f32)

            def lnx():
                LB = O["LB"]
                for u in range(T // LB):
                    rc = pl.ds(pl.multiple_of(tn * T + u * LB, LB), LB)
                    xn2_s[u * LB:(u + 1) * LB, :] = _ln(q_v[rc, :].astype(f32)).astype(bf16)

            def lnz():
                LB = O["LB"]
                for u in range(T // LB):
                    rc = pl.ds(pl.multiple_of(t * T + u * LB, LB), LB)
                    z2_s[rc, :] = _ln(z2f_s[u * LB:(u + 1) * LB, :]).astype(bf16)

            def zdot(c0, c1):
                MB = O["MB"]
                for m in range(T // MB):
                    rm = pl.ds(pl.multiple_of(t * T + m * MB, MB), MB)
                    z = jnp.dot(xn_s[rm, :], win_v[:, c0:c1], preferred_element_type=f32)
                    for cc in range(c0, c1, 128):
                        gz = z[:, cc - c0:cc - c0 + 128]
                        if cc >= FH or not O["late_gelu"]:
                            gz = gelu(gz)
                        if cc >= FH:
                            z2f_s[m * MB:(m + 1) * MB, cc - FH:cc - FH + 128] = gz
                        else:
                            z1_s[rm, cc:cc + 128] = gz.astype(bf16)

            def halo():
                kpad_s[0:HALO, :] = kpad_s[T:T + HALO, :]

            fns = dict(K=kdft, P=kpad, V=kv_chunk, X=xdft, Z=zdot)
            waits = dict(q0=lambda: q_copy(0).wait(), ssm=cs.wait,
                         kv=lambda: (ck.wait(), cv.wait()),
                         q1=lambda: q_copy(tn).wait(),
                         w0=lambda: win_copy(0).wait(), w1=lambda: win_copy(1).wait(),
                         w2=lambda: win_copy(2).wait())

            def body(order):
                for item in order:
                    if item == "lnx":
                        lnx()
                    elif item == "lnz":
                        lnz()
                    elif item == "halo":
                        halo()
                    elif item == "ln0":
                        ln0()
                    elif item == "prefetch":
                        prefetch()
                    elif item in waits:
                        waits[item]()
                    else:
                        fns[item[0]](*item[1:])
                xn_s[rows(tn), :] = xn2_s[...]

            @pl.when(t == 0)
            def _():
                body(O["order0"])

            @pl.when(t > 0)
            def _():
                prefetch()
                cs.wait()
                ck.wait()
                cv.wait()

                @pl.when(t + 1 < NT)
                def _():
                    q_copy(t + 1).wait()

                body(O["order"])

        @pl.when(jnp.logical_and(step >= NT, step < 2 * NT))
        @jax.named_scope('phC1')
        def _():
            t = step - NT
            r = rows(t)
            wsp_copy(t).wait()
            b = bsp_ref[r].astype(f32).reshape(1, T)
            bcol = jnp.transpose(jnp.broadcast_to(b, (128, T)))

            def mac(fb, lt, outs):
                f0 = pl.multiple_of(t * FB + fb * 8, 8)
                fre = pl.ds(f0, 8)
                fim = pl.ds(f0 + _C, 8)
                ls = slice(lt * 128, (lt + 1) * 128)
                for i in outs:
                    are = aim = None
                    for j in range(i + 1):
                        xr = xf_s[j, fre, ls]
                        xi = xf_s[j, fim, ls]
                        kr = kf_s[i - j, fre, ls]
                        ki = kf_s[i - j, fim, ls]
                        if are is None:
                            are = xr * kr - xi * ki
                            aim = xr * ki + xi * kr
                        else:
                            are = are + xr * kr - xi * ki
                            aim = aim + xr * ki + xi * kr
                    sf_s[i, fre, ls] = are
                    sf_s[i, fim, ls] = aim

            groups = _OPT['groups']
            work = [(fb, lt, g_) for fb in range(FB // 8) for lt in range(D // 128) for g_ in groups]
            pace = pl.ds(pl.multiple_of(zero_s[0] * 8, 8), 8)
            KQ = _OPT['KQ']
            nround = (FH // 128) * KQ
            wi = 0
            for c in range(FH // 128):
                cs_ = slice(c * 128, (c + 1) * 128)
                acc = None
                for kq in range(KQ):
                    ks_ = slice(kq * (S // KQ), (kq + 1) * (S // KQ))
                    p = jnp.dot(wsp_v[r, ks_], z2_s[ks_, cs_], preferred_element_type=f32)
                    acc = p if acc is None else acc + p
                    rd = c * KQ + kq
                    hi = -(-len(work) * (rd + 1) // nround)
                    n = hi - wi
                    for q_, w in enumerate(work[wi:hi]):
                        row = (q_ * T // n) // 8 * 8
                        xf_s[NC, pace, 0:128] = p[row:row + 8, :]
                        mac(*w)
                    wi = hi
                z1 = z1_s[r, cs_].astype(f32)
                if _OPT['late_gelu']:
                    z1 = jax.nn.gelu(z1, approximate=True)
                h = z1 * (acc + bcol)
                z1_s[r, cs_] = h.astype(bf16)

        @pl.when(step >= 2 * NT)
        @jax.named_scope('phC2')
        def _():
            t = step - 2 * NT
            r = rows(t)

            @pl.when(t == 0)
            def _():
                wout_copy().wait()

            o = jnp.dot(z1_s[r, :], wout_v[...], preferred_element_type=f32)
            gate = o * jax.nn.sigmoid(o)
            inv = inv_ref[...]
            dvec = dvec_ref[...].astype(f32).reshape(1, D)
            H = _C // 2
            for c in range(CPT):
                i = t * CPT + c
                cur = sf_s[i]
                prv = sf_s[jnp.maximum(i - 1, 0)]
                if c == 0:
                    prv = jnp.where(t > 0, prv, 0.0)
                pre, pim = prv[:_C], prv[_C:]
                add = jnp.concatenate(
                    [-pim[:H], pim[H:], pre[:H], -pre[H:]], axis=0)
                tt = (cur + add).astype(bf16)
                y = jnp.dot(inv, tt, preferred_element_type=f32)
                rc = pl.ds(pl.multiple_of(t * T + c * _C, _C), _C)
                y = y + kv_s[rc, :].astype(f32) * dvec
                s = xn_s[rc, :].astype(f32) * y
                out = q_v[rc, :].astype(f32) + s * gate[c * _C:(c + 1) * _C, :]
                o_ref[c * _C:(c + 1) * _C, :] = out.astype(o_ref.dtype)

    full = lambda shape: pl.BlockSpec(shape, lambda s: (0,) * len(shape))
    anyspec = pl.BlockSpec(memory_space=pl.ANY)
    out = pl.pallas_call(
        kernel,
        grid=(3 * NT,),
        in_specs=[anyspec] * 7 + [
            full((KS, D)), full((D,)), full((S,)),
            full((2 * _C, _C)), full((_C, 2 * _C)),
        ],
        out_specs=pl.BlockSpec((None, T, D),
                               lambda s: (0, jnp.maximum(s - 2 * NT, 0), 0)),
        out_shape=jax.ShapeDtypeStruct((1, S, D), A_q.dtype),
        scratch_shapes=[
            pltpu.VMEM((S + 32, D), bf16), pltpu.VMEM((S, D), bf16),
            pltpu.VMEM((S, D), bf16), pltpu.VMEM((D, S), bf16),
            pltpu.VMEM((D, F2), bf16), pltpu.VMEM((S, S), bf16),
            pltpu.VMEM((FH, D), bf16),
            pltpu.VMEM((S, D), bf16), pltpu.VMEM((S, D), bf16),
            pltpu.VMEM((S, FH), bf16), pltpu.VMEM((S, FH), bf16),
            pltpu.VMEM((NC + 1, 2 * _C, D), f32), pltpu.VMEM((NC, 2 * _C, D), f32),
            pltpu.VMEM((NC, 2 * _C, D), f32),
            pltpu.VMEM((T + HALO + 16, D), f32), pltpu.VMEM((8, D), f32),
            pltpu.VMEM((T + 16, FH), f32), pltpu.VMEM((T, D), bf16),
            pltpu.SMEM((1,), jnp.int32),
            pltpu.SemaphoreType.DMA((7, NT)),
        ],
        compiler_params=pltpu.CompilerParams(
            dimension_semantics=("arbitrary",),
            vmem_limit_bytes=110 * 1024 * 1024,
        ),
    )(A_q, A_k, A_v, A_ssm_k, B_w_in, B_w_sp, B_w_out,
      A_shift_k.T, A_ssm_D, B_b_sp,
      jnp.asarray(_FWD, bf16), jnp.asarray(_INV, bf16))
    return out
```

```python
import numpy as np
import jax
import jax.numpy as jnp
import jax.experimental.pallas as pl
import jax.experimental.pallas.tpu as pltpu

_C = 128


def _dft_mats():
    n = np.arange(_C)
    f = np.concatenate([np.arange(0, _C, 2), np.arange(1, _C, 2)])
    th = 2.0 * np.pi * (f[:, None] + 0.5) * n[None, :] / (2 * _C)
    fwd = np.concatenate([np.cos(th), -np.sin(th)], axis=0)
    inv = np.concatenate([np.cos(th).T, -np.sin(th).T], axis=1) / _C
    return fwd.astype(np.float32), inv.astype(np.float32)


_FWD, _INV = _dft_mats()
_OPT = dict(pad=8, late_gelu=False, KQ=4, groups=[[i] for i in range(16)], RB=32, LB=16, MB=512, order=[
    ("K", 0), ("K", 1), ("K", 2), ("K", 3), ("P", 0), ("P", 1), ("P", 2), ("P", 3),
    ("Z", 1024, 1536), ("V", 0), ("X", 0), ("V", 1), ("X", 1), "lnx",
    ("Z", 512, 1024), ("V", 2), ("X", 2), ("V", 3), ("X", 3), "halo",
    ("Z", 0, 512), "lnz"],
    order0=["q0", "ln0", "w2", ("Z", 1024, 1536), "ssm", ("K", 0), ("K", 1), ("K", 2), ("K", 3),
            "w1", ("Z", 512, 1024), "kv", ("P", 0), ("P", 1), ("P", 2), ("P", 3), "prefetch",
            ("V", 0), ("X", 0), ("V", 1), ("X", 1), ("V", 2), ("X", 2), ("V", 3), ("X", 3), "halo",
            "w0", "q1", ("Z", 0, 512), "lnz", "lnx"])


def _ln(x):
    m = jnp.mean(x, axis=-1, keepdims=True)
    xc = x - m
    v = jnp.mean(xc * xc, axis=-1, keepdims=True)
    return xc * jax.lax.rsqrt(v + 1e-5)


def pallas_recurrent_scan__ssm_conv_h3__mixer_gmlp__prompt_kernel(
    A_q: jax.Array,
    A_k: jax.Array,
    A_v: jax.Array,
    A_shift_k: jax.Array,
    A_ssm_k: jax.Array,
    A_ssm_D: jax.Array,
    B_x: jax.Array,
    B_w_in: jax.Array,
    B_w_sp: jax.Array,
    B_b_sp: jax.Array,
    B_w_out: jax.Array,
):
    del B_x
    _, S, D = A_q.shape
    KS = A_shift_k.shape[-1]
    F2 = B_w_in.shape[-1]
    FH = F2 // 2
    T = 512
    NT = S // T
    CPT = T // _C
    NC = S // _C
    FB = _C // NT
    HALO = 8
    IM = _C + _OPT['pad']
    NW_COLS = 128
    bf16, f32 = jnp.bfloat16, jnp.float32

    def kernel(q_h, k_h, v_h, ssm_h, win_h, wsp_h, wout_h,
               shift_ref, dvec_ref, bsp_ref, fwd_ref, inv_ref,
               o_ref,
               q_v, k_v, v_v, ssm_v, win_v, wsp_v, wout_v,
               xn_s, kv_s, z1_s, z2_s, xf_s, kf_s, sf_s, kpad_s, shift_s, z2f_s, xn2_s, zero_s,
               sems):
        step = pl.program_id(0)

        def rows(t):
            return pl.ds(pl.multiple_of(t * T, T), T)

        def q_copy(t):
            r = rows(t)
            return pltpu.make_async_copy(q_h.at[0, r, :], q_v.at[r, :], sems.at[0, t])

        def tile_copies(t):
            r = rows(t)
            return (
                pltpu.make_async_copy(k_h.at[0, r, :], k_v.at[r, :], sems.at[1, t]),
                pltpu.make_async_copy(v_h.at[0, r, :], v_v.at[r, :], sems.at[2, t]),
                pltpu.make_async_copy(ssm_h.at[:, r], ssm_v.at[:, r], sems.at[3, t]),
            )

        def wsp_copy(t):
            r = rows(t)
            return pltpu.make_async_copy(wsp_h.at[r, :], wsp_v.at[r, :], sems.at[4, t])

        def win_copy(c):
            cs_ = pl.ds(c * 512, 512)
            return pltpu.make_async_copy(win_h.at[:, cs_], win_v.at[:, cs_], sems.at[6, c])

        def wout_copy():
            return pltpu.make_async_copy(wout_h, wout_v, sems.at[5, 1])

        @pl.when(step == 0)
        def _():
            ck, cv, cs = tile_copies(0)
            q_copy(0).start()
            win_copy(2).start()
            cs.start()
            win_copy(1).start()
            ck.start()
            cv.start()
            win_copy(0).start()
            q_copy(1).start()
            kpad_s[0:HALO, :] = jnp.zeros((HALO, D), f32)
            zero_s[0] = 0
            shift_s[0:KS, :] = shift_ref[...].astype(f32)

        @pl.when(step < NT)
        @jax.named_scope('phB')
        def _():
            t = step

            tn = jnp.minimum(t + 1, NT - 1)

            def prefetch():
                @pl.when(t + 1 < NT)
                def _():
                    for c in tile_copies(t + 1):
                        c.start()

                @pl.when(t + 2 < NT)
                def _():
                    q_copy(t + 2).start()

                wsp_copy(t).start()

                @pl.when(t == 1)
                def _():
                    wout_copy().start()

            r = rows(t)
            ck, cv, cs = tile_copies(t)

            def ln0():
                for c in range(T // 16):
                    rc = slice(c * 16, (c + 1) * 16)
                    xn_s[rc, :] = _ln(q_v[rc, :].astype(f32)).astype(bf16)

            fwd = fwd_ref[...]
            O = _OPT

            def kdft(c):
                blk = ssm_v[:, pl.ds(pl.multiple_of(t * T + c * _C, _C), _C)]
                res = jax.lax.dot_general(
                    fwd, blk, (((1,), (1,)), ((), ())), preferred_element_type=f32)
                kf_s[t * CPT + c, 0:_C, :] = res[:_C]
                kf_s[t * CPT + c, IM:IM + _C, :] = res[_C:]

            def gelu(z):
                return jax.nn.gelu(z, approximate=True)

            RB = O["RB"]

            def kpad(c):
                rc = pl.ds(pl.multiple_of(t * T + c * _C, _C), _C)
                kpad_s[HALO + c * _C:HALO + (c + 1) * _C, :] = k_v[rc, :].astype(f32)

            def kv_chunk(c):
                for u in range(_C // RB):
                    o = HALO + c * _C + u * RB
                    ksh = kpad_s[o:o + RB, :] * shift_s[0:1, :]
                    for j in range(1, KS):
                        ksh = ksh + kpad_s[o - j:o - j + RB, :] * shift_s[j:j + 1, :]
                    rc = pl.ds(pl.multiple_of(t * T + c * _C + u * RB, RB), RB)
                    kv_s[rc, :] = (ksh * v_v[rc, :].astype(f32)).astype(bf16)

            def xdft(c):
                rc = pl.ds(pl.multiple_of(t * T + c * _C, _C), _C)
                res = jnp.dot(fwd, kv_s[rc, :], preferred_element_type=f32)
                xf_s[t * CPT + c, 0:_C, :] = res[:_C]
                xf_s[t * CPT + c, IM:IM + _C, :] = res[_C:]

            def lnx():
                LB = O["LB"]
                for u in range(T // LB):
                    rc = pl.ds(pl.multiple_of(tn * T + u * LB, LB), LB)
                    xn2_s[u * LB:(u + 1) * LB, :] = _ln(q_v[rc, :].astype(f32)).astype(bf16)

            def lnz():
                LB = O["LB"]
                for u in range(T // LB):
                    rc = pl.ds(pl.multiple_of(t * T + u * LB, LB), LB)
                    z2_s[rc, :] = _ln(z2f_s[u * LB:(u + 1) * LB, :]).astype(bf16)

            def zdot(c0, c1):
                MB = O["MB"]
                for m in range(T // MB):
                    rm = pl.ds(pl.multiple_of(t * T + m * MB, MB), MB)
                    z = jnp.dot(xn_s[rm, :], win_v[:, c0:c1], preferred_element_type=f32)
                    for cc in range(c0, c1, 128):
                        gz = z[:, cc - c0:cc - c0 + 128]
                        if cc >= FH or not O["late_gelu"]:
                            gz = gelu(gz)
                        if cc >= FH:
                            z2f_s[m * MB:(m + 1) * MB, cc - FH:cc - FH + 128] = gz
                        else:
                            z1_s[rm, cc:cc + 128] = gz.astype(bf16)

            def halo():
                kpad_s[0:HALO, :] = kpad_s[T:T + HALO, :]

            fns = dict(K=kdft, P=kpad, V=kv_chunk, X=xdft, Z=zdot)
            waits = dict(q0=lambda: q_copy(0).wait(), ssm=cs.wait,
                         kv=lambda: (ck.wait(), cv.wait()),
                         q1=lambda: q_copy(tn).wait(),
                         w0=lambda: win_copy(0).wait(), w1=lambda: win_copy(1).wait(),
                         w2=lambda: win_copy(2).wait())

            def body(order):
                for item in order:
                    if item == "lnx":
                        lnx()
                    elif item == "lnz":
                        lnz()
                    elif item == "halo":
                        halo()
                    elif item == "ln0":
                        ln0()
                    elif item == "prefetch":
                        prefetch()
                    elif item in waits:
                        waits[item]()
                    else:
                        fns[item[0]](*item[1:])
                xn_s[rows(tn), :] = xn2_s[...]

            @pl.when(t == 0)
            def _():
                body(O["order0"])

            @pl.when(t > 0)
            def _():
                prefetch()
                cs.wait()
                ck.wait()
                cv.wait()

                @pl.when(t + 1 < NT)
                def _():
                    q_copy(t + 1).wait()

                body(O["order"])

        @pl.when(jnp.logical_and(step >= NT, step < 2 * NT))
        @jax.named_scope('phC1')
        def _():
            t = step - NT
            r = rows(t)
            wsp_copy(t).wait()
            b = bsp_ref[r].astype(f32).reshape(1, T)
            bcol = jnp.transpose(jnp.broadcast_to(b, (128, T)))

            def mac(fb, lt, outs):
                f0 = pl.multiple_of(t * FB + fb * 8, 8)
                fre = pl.ds(f0, 8)
                fim = pl.ds(f0 + IM, 8)
                ls = slice(lt * 128, (lt + 1) * 128)
                for i in outs:
                    are = aim = None
                    for j in range(i + 1):
                        xr = xf_s[j, fre, ls]
                        xi = xf_s[j, fim, ls]
                        kr = kf_s[i - j, fre, ls]
                        ki = kf_s[i - j, fim, ls]
                        if are is None:
                            are = xr * kr - xi * ki
                            aim = xr * ki + xi * kr
                        else:
                            are = are + xr * kr - xi * ki
                            aim = aim + xr * ki + xi * kr
                    sf_s[i, fre, ls] = are
                    sf_s[i, fim, ls] = aim

            groups = _OPT['groups']
            work = [(fb, lt, g_) for fb in range(FB // 8) for lt in range(D // 128) for g_ in groups]
            pace = pl.ds(pl.multiple_of(zero_s[0] * 8, 8), 8)
            KQ = _OPT['KQ']
            nround = (FH // 128) * KQ
            wi = 0
            for c in range(FH // 128):
                cs_ = slice(c * 128, (c + 1) * 128)
                acc = None
                for kq in range(KQ):
                    ks_ = slice(kq * (S // KQ), (kq + 1) * (S // KQ))
                    p = jnp.dot(wsp_v[r, ks_], z2_s[ks_, cs_], preferred_element_type=f32)
                    acc = p if acc is None else acc + p
                    rd = c * KQ + kq
                    hi = -(-len(work) * (rd + 1) // nround)
                    n = hi - wi
                    for q_, w in enumerate(work[wi:hi]):
                        row = (q_ * T // n) // 8 * 8
                        xf_s[NC, pace, 0:128] = p[row:row + 8, :]
                        mac(*w)
                    wi = hi
                z1 = z1_s[r, cs_].astype(f32)
                if _OPT['late_gelu']:
                    z1 = jax.nn.gelu(z1, approximate=True)
                h = z1 * (acc + bcol)
                z1_s[r, cs_] = h.astype(bf16)

        @pl.when(step >= 2 * NT)
        @jax.named_scope('phC2')
        def _():
            t = step - 2 * NT
            r = rows(t)

            @pl.when(t == 0)
            def _():
                wout_copy().wait()

            o = jnp.dot(z1_s[r, :], wout_v[...], preferred_element_type=f32)
            gate = o * jax.nn.sigmoid(o)
            inv = inv_ref[...]
            dvec = dvec_ref[...].astype(f32).reshape(1, D)
            H = _C // 2
            for c in range(CPT):
                i = t * CPT + c
                cur = jnp.concatenate([sf_s[i, 0:_C, :], sf_s[i, IM:IM + _C, :]], axis=0)
                ip = jnp.maximum(i - 1, 0)
                pre, pim = sf_s[ip, 0:_C, :], sf_s[ip, IM:IM + _C, :]
                if c == 0:
                    pre = jnp.where(t > 0, pre, 0.0)
                    pim = jnp.where(t > 0, pim, 0.0)
                add = jnp.concatenate(
                    [-pim[:H], pim[H:], pre[:H], -pre[H:]], axis=0)
                tt = (cur + add).astype(bf16)
                y = jnp.dot(inv, tt, preferred_element_type=f32)
                rc = pl.ds(pl.multiple_of(t * T + c * _C, _C), _C)
                y = y + kv_s[rc, :].astype(f32) * dvec
                s = xn_s[rc, :].astype(f32) * y
                out = q_v[rc, :].astype(f32) + s * gate[c * _C:(c + 1) * _C, :]
                o_ref[c * _C:(c + 1) * _C, :] = out.astype(o_ref.dtype)

    full = lambda shape: pl.BlockSpec(shape, lambda s: (0,) * len(shape))
    anyspec = pl.BlockSpec(memory_space=pl.ANY)
    out = pl.pallas_call(
        kernel,
        grid=(3 * NT,),
        in_specs=[anyspec] * 7 + [
            full((KS, D)), full((D,)), full((S,)),
            full((2 * _C, _C)), full((_C, 2 * _C)),
        ],
        out_specs=pl.BlockSpec((None, T, D),
                               lambda s: (0, jnp.maximum(s - 2 * NT, 0), 0)),
        out_shape=jax.ShapeDtypeStruct((1, S, D), A_q.dtype),
        scratch_shapes=[
            pltpu.VMEM((S + 32, D), bf16), pltpu.VMEM((S, D), bf16),
            pltpu.VMEM((S, D), bf16), pltpu.VMEM((D, S), bf16),
            pltpu.VMEM((D, F2), bf16), pltpu.VMEM((S, S), bf16),
            pltpu.VMEM((FH, D), bf16),
            pltpu.VMEM((S, D), bf16), pltpu.VMEM((S, D), bf16),
            pltpu.VMEM((S, FH), bf16), pltpu.VMEM((S, FH), bf16),
            pltpu.VMEM((NC + 1, IM + _C, D), f32), pltpu.VMEM((NC, IM + _C, D), f32),
            pltpu.VMEM((NC, IM + _C, D), f32),
            pltpu.VMEM((T + HALO + 16, D), f32), pltpu.VMEM((8, D), f32),
            pltpu.VMEM((T + 16, FH), f32), pltpu.VMEM((T, D), bf16),
            pltpu.SMEM((1,), jnp.int32),
            pltpu.SemaphoreType.DMA((7, NT)),
        ],
        compiler_params=pltpu.CompilerParams(
            dimension_semantics=("arbitrary",),
            vmem_limit_bytes=110 * 1024 * 1024,
        ),
    )(A_q, A_k, A_v, A_ssm_k, B_w_in, B_w_sp, B_w_out,
      A_shift_k.T, A_ssm_D, B_b_sp,
      jnp.asarray(_FWD, bf16), jnp.asarray(_INV, bf16))
    return out
```

```python
import numpy as np
import jax
import jax.numpy as jnp
import jax.experimental.pallas as pl
import jax.experimental.pallas.tpu as pltpu

_C = 128


def _dft_mats():
    n = np.arange(_C)
    f = np.concatenate([np.arange(0, _C, 2), np.arange(1, _C, 2)])
    th = 2.0 * np.pi * (f[:, None] + 0.5) * n[None, :] / (2 * _C)
    fwd = np.concatenate([np.cos(th), -np.sin(th)], axis=0)
    inv = np.concatenate([np.cos(th).T, -np.sin(th).T], axis=1) / _C
    return fwd.astype(np.float32), inv.astype(np.float32)


_FWD, _INV = _dft_mats()
_OPT = dict(NR=4, RBp=32, G=6, iorder=list(range(16)), pad=8, late_gelu=False, KQ=4, groups=[[i] for i in range(16)], RB=32, LB=16, MB=512, order=[
    ("K", 0), ("K", 1), ("K", 2), ("K", 3), ("P", 0), ("P", 1), ("P", 2), ("P", 3),
    ("Z", 1024, 1536), ("V", 0), ("X", 0), ("V", 1), ("X", 1), "lnx",
    ("Z", 512, 1024), ("V", 2), ("X", 2), ("V", 3), ("X", 3), "halo",
    ("Z", 0, 512), "lnz"],
    order0=["q0", "ln0", "w2", ("Z", 1024, 1536), "ssm", ("K", 0), ("K", 1), ("K", 2), ("K", 3),
            "w1", ("Z", 512, 1024), "kv", ("P", 0), ("P", 1), ("P", 2), ("P", 3), "prefetch",
            ("V", 0), ("X", 0), ("V", 1), ("X", 1), ("V", 2), ("X", 2), ("V", 3), ("X", 3), "halo",
            "w0", "q1", ("Z", 0, 512), "lnz", "lnx"])


def _ln(x):
    m = jnp.mean(x, axis=-1, keepdims=True)
    xc = x - m
    v = jnp.mean(xc * xc, axis=-1, keepdims=True)
    return xc * jax.lax.rsqrt(v + 1e-5)


def pallas_recurrent_scan__ssm_conv_h3__mixer_gmlp__prompt_kernel(
    A_q: jax.Array,
    A_k: jax.Array,
    A_v: jax.Array,
    A_shift_k: jax.Array,
    A_ssm_k: jax.Array,
    A_ssm_D: jax.Array,
    B_x: jax.Array,
    B_w_in: jax.Array,
    B_w_sp: jax.Array,
    B_b_sp: jax.Array,
    B_w_out: jax.Array,
):
    del B_x
    _, S, D = A_q.shape
    KS = A_shift_k.shape[-1]
    F2 = B_w_in.shape[-1]
    FH = F2 // 2
    T = 512
    NT = S // T
    CPT = T // _C
    NC = S // _C
    FB = _C // NT
    HALO = 8
    IM = _C + _OPT['pad']
    NW_COLS = 128
    bf16, f32 = jnp.bfloat16, jnp.float32

    def kernel(q_h, k_h, v_h, ssm_h, win_h, wsp_h, wout_h,
               shift_ref, dvec_ref, bsp_ref, fwd_ref, inv_ref,
               o_ref,
               q_v, k_v, v_v, ssm_v, win_v, wsp_v, wout_v,
               xn_s, kv_s, z1_s, z2_s, xf_s, kf_s, sf_s, kpad_s, shift_s, z2f_s, xn2_s, zero_s,
               sems):
        step = pl.program_id(0)

        def rows(t):
            return pl.ds(pl.multiple_of(t * T, T), T)

        def q_copy(t):
            r = rows(t)
            return pltpu.make_async_copy(q_h.at[0, r, :], q_v.at[r, :], sems.at[0, t])

        def tile_copies(t):
            r = rows(t)
            return (
                pltpu.make_async_copy(k_h.at[0, r, :], k_v.at[r, :], sems.at[1, t]),
                pltpu.make_async_copy(v_h.at[0, r, :], v_v.at[r, :], sems.at[2, t]),
                pltpu.make_async_copy(ssm_h.at[:, r], ssm_v.at[:, r], sems.at[3, t]),
            )

        def wsp_copy(t):
            r = rows(t)
            return pltpu.make_async_copy(wsp_h.at[r, :], wsp_v.at[r, :], sems.at[4, t])

        def win_copy(c):
            cs_ = pl.ds(c * 512, 512)
            return pltpu.make_async_copy(win_h.at[:, cs_], win_v.at[:, cs_], sems.at[6, c])

        def wout_copy():
            return pltpu.make_async_copy(wout_h, wout_v, sems.at[5, 1])

        @pl.when(step == 0)
        def _():
            ck, cv, cs = tile_copies(0)
            q_copy(0).start()
            win_copy(2).start()
            cs.start()
            win_copy(1).start()
            ck.start()
            cv.start()
            win_copy(0).start()
            q_copy(1).start()
            kpad_s[0:HALO, :] = jnp.zeros((HALO, D), f32)
            zero_s[0] = 0
            shift_s[0:KS, :] = shift_ref[...].astype(f32)

        @pl.when(step < NT)
        @jax.named_scope('phB')
        def _():
            t = step

            tn = jnp.minimum(t + 1, NT - 1)

            def prefetch():
                @pl.when(t + 1 < NT)
                def _():
                    for c in tile_copies(t + 1):
                        c.start()

                @pl.when(t + 2 < NT)
                def _():
                    q_copy(t + 2).start()

                wsp_copy(t).start()

                @pl.when(t == 1)
                def _():
                    wout_copy().start()

            r = rows(t)
            ck, cv, cs = tile_copies(t)

            def ln0():
                for c in range(T // 16):
                    rc = slice(c * 16, (c + 1) * 16)
                    xn_s[rc, :] = _ln(q_v[rc, :].astype(f32)).astype(bf16)

            fwd = fwd_ref[...]
            O = _OPT

            def kdft(c):
                blk = ssm_v[:, pl.ds(pl.multiple_of(t * T + c * _C, _C), _C)]
                res = jax.lax.dot_general(
                    fwd, blk, (((1,), (1,)), ((), ())), preferred_element_type=f32)
                kf_s[t * CPT + c, 0:_C, :] = res[:_C]
                kf_s[t * CPT + c, IM:IM + _C, :] = res[_C:]

            def gelu(z):
                return jax.nn.gelu(z, approximate=True)

            RB = O["RB"]

            def kpad(c):
                rc = pl.ds(pl.multiple_of(t * T + c * _C, _C), _C)
                kpad_s[HALO + c * _C:HALO + (c + 1) * _C, :] = k_v[rc, :].astype(f32)

            def kv_chunk(c):
                for u in range(_C // RB):
                    o = HALO + c * _C + u * RB
                    ksh = kpad_s[o:o + RB, :] * shift_s[0:1, :]
                    for j in range(1, KS):
                        ksh = ksh + kpad_s[o - j:o - j + RB, :] * shift_s[j:j + 1, :]
                    rc = pl.ds(pl.multiple_of(t * T + c * _C + u * RB, RB), RB)
                    kv_s[rc, :] = (ksh * v_v[rc, :].astype(f32)).astype(bf16)

            def xdft(c):
                rc = pl.ds(pl.multiple_of(t * T + c * _C, _C), _C)
                res = jnp.dot(fwd, kv_s[rc, :], preferred_element_type=f32)
                xf_s[t * CPT + c, 0:_C, :] = res[:_C]
                xf_s[t * CPT + c, IM:IM + _C, :] = res[_C:]

            def lnx():
                LB = O["LB"]
                for u in range(T // LB):
                    rc = pl.ds(pl.multiple_of(tn * T + u * LB, LB), LB)
                    xn2_s[u * LB:(u + 1) * LB, :] = _ln(q_v[rc, :].astype(f32)).astype(bf16)

            def lnz():
                LB = O["LB"]
                for u in range(T // LB):
                    rc = pl.ds(pl.multiple_of(t * T + u * LB, LB), LB)
                    z2_s[rc, :] = _ln(z2f_s[u * LB:(u + 1) * LB, :]).astype(bf16)

            def zdot(c0, c1):
                MB = O["MB"]
                for m in range(T // MB):
                    rm = pl.ds(pl.multiple_of(t * T + m * MB, MB), MB)
                    z = jnp.dot(xn_s[rm, :], win_v[:, c0:c1], preferred_element_type=f32)
                    for cc in range(c0, c1, 128):
                        gz = z[:, cc - c0:cc - c0 + 128]
                        if cc >= FH or not O["late_gelu"]:
                            gz = gelu(gz)
                        if cc >= FH:
                            z2f_s[m * MB:(m + 1) * MB, cc - FH:cc - FH + 128] = gz
                        else:
                            z1_s[rm, cc:cc + 128] = gz.astype(bf16)

            zo = zero_s[0]
            pc_k = pl.ds(pl.multiple_of(HALO + T + zo * 8, 8), 8)
            pc_z = pl.ds(pl.multiple_of(T + zo * 8, 8), 8)
            pc_q = pl.ds(pl.multiple_of(S + zo * 16, 16), 16)

            def pieces(kind):
                LB = 16
                if kind == "lnx":
                    def f(u, val):
                        q_v[pc_q, 0:128] = val.astype(bf16)
                        rc = pl.ds(pl.multiple_of(tn * T + u * LB, LB), LB)
                        xn2_s[u * LB:(u + 1) * LB, :] = _ln(q_v[rc, :].astype(f32)).astype(bf16)
                    return [(f, u) for u in range(T // LB)]
                if kind == "lnz":
                    def f(u, val):
                        z2f_s[pc_z, 0:128] = val[0:8]
                        rc = pl.ds(pl.multiple_of(t * T + u * LB, LB), LB)
                        z2_s[rc, :] = _ln(z2f_s[u * LB:(u + 1) * LB, :]).astype(bf16)
                    return [(f, u) for u in range(T // LB)]
                RBp = O["RBp"]

                def f(u, val):
                    kpad_s[pc_k, 0:128] = val[0:8]
                    o = HALO + u * RBp
                    ksh = kpad_s[o:o + RBp, :] * shift_s[0:1, :]
                    for j in range(1, KS):
                        ksh = ksh + kpad_s[o - j:o - j + RBp, :] * shift_s[j:j + 1, :]
                    rc = pl.ds(pl.multiple_of(t * T + u * RBp, RBp), RBp)
                    kv_s[rc, :] = (ksh * v_v[rc, :].astype(f32)).astype(bf16)
                return [(f, u) for u in range(T // RBp)]

            def zpaced(c0, c1, kind):
                wk = pieces(kind)
                NR = O["NR"]
                acc = None
                wi = 0
                for kt in range(D // 128):
                    ks_ = slice(kt * 128, (kt + 1) * 128)
                    p_ = jnp.dot(xn_s[r, ks_], win_v[ks_, c0:c1], preferred_element_type=f32)
                    acc = p_ if acc is None else acc + p_
                    hi = min(len(wk), -(-len(wk) * (kt + 1) // NR))
                    n = hi - wi
                    for q_, (f, u) in enumerate(wk[wi:hi]):
                        row = (q_ * T // n) // 16 * 16
                        f(u, p_[row:row + 16, 0:128])
                    wi = hi
                for cc in range(c0, c1, 128):
                    gz = gelu(acc[:, cc - c0:cc - c0 + 128])
                    if cc >= FH:
                        z2f_s[0:T, cc - FH:cc - FH + 128] = gz
                    else:
                        z1_s[r, cc:cc + 128] = gz.astype(bf16)

            def halo():
                kpad_s[0:HALO, :] = kpad_s[T:T + HALO, :]

            fns = dict(K=kdft, P=kpad, V=kv_chunk, X=xdft, Z=zdot, Y=zpaced)
            waits = dict(q0=lambda: q_copy(0).wait(), ssm=cs.wait,
                         kv=lambda: (ck.wait(), cv.wait()),
                         q1=lambda: q_copy(tn).wait(),
                         w0=lambda: win_copy(0).wait(), w1=lambda: win_copy(1).wait(),
                         w2=lambda: win_copy(2).wait())

            def body(order):
                for item in order:
                    if item == "lnx":
                        lnx()
                    elif item == "lnz":
                        lnz()
                    elif item == "halo":
                        halo()
                    elif item == "ln0":
                        ln0()
                    elif item == "prefetch":
                        prefetch()
                    elif item in waits:
                        waits[item]()
                    else:
                        fns[item[0]](*item[1:])
                xn_s[rows(tn), :] = xn2_s[...]

            @pl.when(t == 0)
            def _():
                body(O["order0"])

            @pl.when(t > 0)
            def _():
                prefetch()
                cs.wait()
                ck.wait()
                cv.wait()

                @pl.when(t + 1 < NT)
                def _():
                    q_copy(t + 1).wait()

                body(O["order"])

        @pl.when(jnp.logical_and(step >= NT, step < 2 * NT))
        @jax.named_scope('phC1')
        def _():
            t = step - NT
            r = rows(t)
            wsp_copy(t).wait()
            b = bsp_ref[r].astype(f32).reshape(1, T)
            bcol = jnp.transpose(jnp.broadcast_to(b, (128, T)))

            terms = [(fb, lt, i, j) for fb in range(FB // 8) for lt in range(D // 128)
                     for i in _OPT['iorder'] for j in range(i + 1)]
            G = _OPT['G']
            work = [terms[u:u + G] for u in range(0, len(terms), G)]
            acc_c = [None, None]

            def mac(piece):
                for fb, lt, i, j in piece:
                    f0 = pl.multiple_of(t * FB + fb * 8, 8)
                    fre = pl.ds(f0, 8)
                    fim = pl.ds(f0 + IM, 8)
                    ls = slice(lt * 128, (lt + 1) * 128)
                    xr = xf_s[j, fre, ls]
                    xi = xf_s[j, fim, ls]
                    kr = kf_s[i - j, fre, ls]
                    ki = kf_s[i - j, fim, ls]
                    if j == 0:
                        are = xr * kr - xi * ki
                        aim = xr * ki + xi * kr
                    else:
                        are = acc_c[0] + xr * kr - xi * ki
                        aim = acc_c[1] + xr * ki + xi * kr
                    acc_c[0], acc_c[1] = are, aim
                    if j == i:
                        sf_s[i, fre, ls] = are
                        sf_s[i, fim, ls] = aim

            pace = pl.ds(pl.multiple_of(zero_s[0] * 8, 8), 8)
            KQ = _OPT['KQ']
            nround = (FH // 128) * KQ
            wi = 0
            for c in range(FH // 128):
                cs_ = slice(c * 128, (c + 1) * 128)
                acc = None
                for kq in range(KQ):
                    ks_ = slice(kq * (S // KQ), (kq + 1) * (S // KQ))
                    p = jnp.dot(wsp_v[r, ks_], z2_s[ks_, cs_], preferred_element_type=f32)
                    acc = p if acc is None else acc + p
                    rd = c * KQ + kq
                    hi = -(-len(work) * (rd + 1) // nround)
                    n = hi - wi
                    for q_, w in enumerate(work[wi:hi]):
                        row = (q_ * T // n) // 8 * 8
                        xf_s[NC, pace, 0:128] = p[row:row + 8, :]
                        mac(w)
                    wi = hi
                h = z1_s[r, cs_].astype(f32) * (acc + bcol)
                z1_s[r, cs_] = h.astype(bf16)

        @pl.when(step >= 2 * NT)
        @jax.named_scope('phC2')
        def _():
            t = step - 2 * NT
            r = rows(t)

            @pl.when(t == 0)
            def _():
                wout_copy().wait()

            o = jnp.dot(z1_s[r, :], wout_v[...], preferred_element_type=f32)
            gate = o * jax.nn.sigmoid(o)
            inv = inv_ref[...]
            dvec = dvec_ref[...].astype(f32).reshape(1, D)
            H = _C // 2
            for c in range(CPT):
                i = t * CPT + c
                cur = jnp.concatenate([sf_s[i, 0:_C, :], sf_s[i, IM:IM + _C, :]], axis=0)
                ip = jnp.maximum(i - 1, 0)
                pre, pim = sf_s[ip, 0:_C, :], sf_s[ip, IM:IM + _C, :]
                if c == 0:
                    pre = jnp.where(t > 0, pre, 0.0)
                    pim = jnp.where(t > 0, pim, 0.0)
                add = jnp.concatenate(
                    [-pim[:H], pim[H:], pre[:H], -pre[H:]], axis=0)
                tt = (cur + add).astype(bf16)
                y = jnp.dot(inv, tt, preferred_element_type=f32)
                rc = pl.ds(pl.multiple_of(t * T + c * _C, _C), _C)
                y = y + kv_s[rc, :].astype(f32) * dvec
                s = xn_s[rc, :].astype(f32) * y
                out = q_v[rc, :].astype(f32) + s * gate[c * _C:(c + 1) * _C, :]
                o_ref[c * _C:(c + 1) * _C, :] = out.astype(o_ref.dtype)

    full = lambda shape: pl.BlockSpec(shape, lambda s: (0,) * len(shape))
    anyspec = pl.BlockSpec(memory_space=pl.ANY)
    out = pl.pallas_call(
        kernel,
        grid=(3 * NT,),
        in_specs=[anyspec] * 7 + [
            full((KS, D)), full((D,)), full((S,)),
            full((2 * _C, _C)), full((_C, 2 * _C)),
        ],
        out_specs=pl.BlockSpec((None, T, D),
                               lambda s: (0, jnp.maximum(s - 2 * NT, 0), 0)),
        out_shape=jax.ShapeDtypeStruct((1, S, D), A_q.dtype),
        scratch_shapes=[
            pltpu.VMEM((S + 32, D), bf16), pltpu.VMEM((S, D), bf16),
            pltpu.VMEM((S, D), bf16), pltpu.VMEM((D, S), bf16),
            pltpu.VMEM((D, F2), bf16), pltpu.VMEM((S, S), bf16),
            pltpu.VMEM((FH, D), bf16),
            pltpu.VMEM((S, D), bf16), pltpu.VMEM((S, D), bf16),
            pltpu.VMEM((S, FH), bf16), pltpu.VMEM((S, FH), bf16),
            pltpu.VMEM((NC + 1, IM + _C, D), f32), pltpu.VMEM((NC, IM + _C, D), f32),
            pltpu.VMEM((NC, IM + _C, D), f32),
            pltpu.VMEM((T + HALO + 16, D), f32), pltpu.VMEM((8, D), f32),
            pltpu.VMEM((T + 16, FH), f32), pltpu.VMEM((T, D), bf16),
            pltpu.SMEM((1,), jnp.int32),
            pltpu.SemaphoreType.DMA((7, NT)),
        ],
        compiler_params=pltpu.CompilerParams(
            dimension_semantics=("arbitrary",),
            vmem_limit_bytes=110 * 1024 * 1024,
        ),
    )(A_q, A_k, A_v, A_ssm_k, B_w_in, B_w_sp, B_w_out,
      A_shift_k.T, A_ssm_D, B_b_sp,
      jnp.asarray(_FWD, bf16), jnp.asarray(_INV, bf16))
    return out
```

```python
import numpy as np
import jax
import jax.numpy as jnp
import jax.experimental.pallas as pl
import jax.experimental.pallas.tpu as pltpu

_C = 128


def _dft_mats():
    n = np.arange(_C)
    f = np.concatenate([np.arange(0, _C, 2), np.arange(1, _C, 2)])
    th = 2.0 * np.pi * (f[:, None] + 0.5) * n[None, :] / (2 * _C)
    fwd = np.concatenate([np.cos(th), -np.sin(th)], axis=0)
    inv = np.concatenate([np.cos(th).T, -np.sin(th).T], axis=1) / _C
    return fwd.astype(np.float32), inv.astype(np.float32)


_FWD, _INV = _dft_mats()
_OPT = dict(NR=4, RBp=32, G=5, iorder=list(range(16)), pad=8, late_gelu=False, KQ=4, groups=[[i] for i in range(16)], RB=32, LB=16, MB=512, order=[
    ("K", 0), ("K", 1), ("K", 2), ("K", 3), ("P", 0), ("P", 1), ("P", 2), ("P", 3),
    ("Z", 1024, 1536), ("V", 0), ("X", 0), ("V", 1), ("X", 1), "lnx",
    ("Z", 512, 1024), ("V", 2), ("X", 2), ("V", 3), ("X", 3), "halo",
    ("Z", 0, 512), "lnz"],
    order0=["q0", "ln0", "w2", ("Z", 1024, 1536), "ssm", ("K", 0), ("K", 1), ("K", 2), ("K", 3),
            "w1", ("Z", 512, 1024), "kv", ("P", 0), ("P", 1), ("P", 2), ("P", 3), "prefetch",
            ("V", 0), ("X", 0), ("V", 1), ("X", 1), ("V", 2), ("X", 2), ("V", 3), ("X", 3), "halo",
            "w0", "q1", ("Z", 0, 512), "lnz", "lnx"])


_G1 = float(np.sqrt(2.0 / np.pi))
_G2 = float(np.sqrt(2.0 / np.pi) * 0.044715)


def _gelu(x):
    h = 0.5 * x
    return h + h * jnp.tanh(x * (_G1 + _G2 * (x * x)))


def _ln(x):
    m = jnp.mean(x, axis=-1, keepdims=True)
    xc = x - m
    v = jnp.mean(xc * xc, axis=-1, keepdims=True)
    return xc * jax.lax.rsqrt(v + 1e-5)


def pallas_recurrent_scan__ssm_conv_h3__mixer_gmlp__prompt_kernel(
    A_q: jax.Array,
    A_k: jax.Array,
    A_v: jax.Array,
    A_shift_k: jax.Array,
    A_ssm_k: jax.Array,
    A_ssm_D: jax.Array,
    B_x: jax.Array,
    B_w_in: jax.Array,
    B_w_sp: jax.Array,
    B_b_sp: jax.Array,
    B_w_out: jax.Array,
):
    del B_x
    _, S, D = A_q.shape
    KS = A_shift_k.shape[-1]
    F2 = B_w_in.shape[-1]
    FH = F2 // 2
    T = 512
    NT = S // T
    CPT = T // _C
    NC = S // _C
    FB = _C // NT
    HALO = 8
    IM = _C + _OPT['pad']
    NW_COLS = 128
    bf16, f32 = jnp.bfloat16, jnp.float32

    def kernel(q_h, k_h, v_h, ssm_h, win_h, wsp_h, wout_h,
               shift_ref, dvec_ref, bsp_ref, fwd_ref, inv_ref,
               o_ref,
               q_v, k_v, v_v, ssm_v, win_v, wsp_v, wout_v,
               xn_s, kv_s, z1_s, z2_s, xf_s, kf_s, sf_s, kpad_s, shift_s, z2f_s, xn2_s, zero_s,
               sems):
        step = pl.program_id(0)

        def rows(t):
            return pl.ds(pl.multiple_of(t * T, T), T)

        def hrows(r0, n):
            if isinstance(r0, int):
                return slice(r0 // 2, (r0 + n) // 2)
            return pl.ds(pl.multiple_of(r0 // 2, n // 2), n // 2)

        def st(ref, r0, val, cs=slice(None)):
            ref[hrows(r0, val.shape[0]), cs] = pltpu.bitcast(val, jnp.uint32)

        def ld(ref, r0, n, cs=slice(None)):
            return pltpu.bitcast(ref[hrows(r0, n), cs], bf16)

        def q_copy(t):
            r = rows(t)
            return pltpu.make_async_copy(q_h.at[0, r, :], q_v.at[r, :], sems.at[0, t])

        def tile_copies(t):
            r = rows(t)
            return (
                pltpu.make_async_copy(k_h.at[0, r, :], k_v.at[r, :], sems.at[1, t]),
                pltpu.make_async_copy(v_h.at[0, r, :], v_v.at[r, :], sems.at[2, t]),
                pltpu.make_async_copy(ssm_h.at[:, r], ssm_v.at[:, r], sems.at[3, t]),
            )

        def wsp_copy(t):
            r = rows(t)
            return [pltpu.make_async_copy(wsp_h.at[r, k * 128:(k + 1) * 128], wsp_v.bitcast(bf16).at[k, r, :],
                                          sems.at[4, t]) for k in range(S // 128)]

        def win_copy(c):
            cs_ = pl.ds(c * 512, 512)
            return pltpu.make_async_copy(win_h.at[:, cs_], win_v.at[:, cs_], sems.at[6, c])

        def wout_copy():
            return pltpu.make_async_copy(wout_h, wout_v, sems.at[5, 1])

        @pl.when(step == 0)
        def _():
            ck, cv, cs = tile_copies(0)
            q_copy(0).start()
            win_copy(2).start()
            cs.start()
            win_copy(1).start()
            ck.start()
            cv.start()
            win_copy(0).start()
            q_copy(1).start()
            kpad_s[0:HALO, :] = jnp.zeros((HALO, D), f32)
            zero_s[0] = 0
            shift_s[0:KS, :] = shift_ref[...].astype(f32)

        @pl.when(step < NT)
        @jax.named_scope('phB')
        def _():
            t = step

            tn = jnp.minimum(t + 1, NT - 1)

            def prefetch():
                @pl.when(t + 1 < NT)
                def _():
                    for c in tile_copies(t + 1):
                        c.start()

                @pl.when(t + 2 < NT)
                def _():
                    q_copy(t + 2).start()

                for c in wsp_copy(t):
                    c.start()

                @pl.when(t == 1)
                def _():
                    wout_copy().start()

            r = rows(t)
            ck, cv, cs = tile_copies(t)

            def ln0():
                for c in range(T // 16):
                    rc = slice(c * 16, (c + 1) * 16)
                    st(xn_s, c * 16, _ln(q_v[rc, :].astype(f32)).astype(bf16))

            fwd = fwd_ref[...]
            O = _OPT

            def kdft(c):
                blk = ssm_v[:, pl.ds(pl.multiple_of(t * T + c * _C, _C), _C)]
                res = jax.lax.dot_general(
                    fwd, blk, (((1,), (1,)), ((), ())), preferred_element_type=f32)
                kf_s[t * CPT + c, 0:_C, :] = res[:_C]
                kf_s[t * CPT + c, IM:IM + _C, :] = res[_C:]

            def gelu(z):
                return _gelu(z)

            RB = O["RB"]

            def kpad(c):
                rc = pl.ds(pl.multiple_of(t * T + c * _C, _C), _C)
                kpad_s[HALO + c * _C:HALO + (c + 1) * _C, :] = k_v[rc, :].astype(f32)

            def kv_chunk(c):
                for u in range(_C // RB):
                    o = HALO + c * _C + u * RB
                    ksh = kpad_s[o:o + RB, :] * shift_s[0:1, :]
                    for j in range(1, KS):
                        ksh = ksh + kpad_s[o - j:o - j + RB, :] * shift_s[j:j + 1, :]
                    rc = pl.ds(pl.multiple_of(t * T + c * _C + u * RB, RB), RB)
                    st(kv_s, t * T + (o - HALO), (ksh * v_v[rc, :].astype(f32)).astype(bf16))

            def xdft(c):
                rc = pl.ds(pl.multiple_of(t * T + c * _C, _C), _C)
                res = jnp.dot(fwd, ld(kv_s, t * T + c * _C, _C), preferred_element_type=f32)
                xf_s[t * CPT + c, 0:_C, :] = res[:_C]
                xf_s[t * CPT + c, IM:IM + _C, :] = res[_C:]

            def lnx():
                LB = O["LB"]
                for u in range(T // LB):
                    rc = pl.ds(pl.multiple_of(tn * T + u * LB, LB), LB)
                    st(xn2_s, u * LB, _ln(q_v[rc, :].astype(f32)).astype(bf16))

            def lnz():
                LB = O["LB"]
                for u in range(T // LB):
                    rc = pl.ds(pl.multiple_of(t * T + u * LB, LB), LB)
                    st(z2_s, t * T + u * LB, _ln(z2f_s[u * LB:(u + 1) * LB, :]).astype(bf16))

            def zdot(c0, c1):
                MB = O["MB"]
                for m in range(T // MB):
                    rm = pl.ds(pl.multiple_of(t * T + m * MB, MB), MB)
                    z = jnp.dot(ld(xn_s, t * T + m * MB, MB), win_v[:, c0:c1], preferred_element_type=f32)
                    for cc in range(c0, c1, 128):
                        gz = z[:, cc - c0:cc - c0 + 128]
                        if cc >= FH or not O["late_gelu"]:
                            gz = gelu(gz)
                        if cc >= FH:
                            z2f_s[m * MB:(m + 1) * MB, cc - FH:cc - FH + 128] = gz
                        else:
                            st(z1_s, t * T + m * MB, gz.astype(bf16), slice(cc, cc + 128))

            zo = zero_s[0]
            pc_k = pl.ds(pl.multiple_of(HALO + T + zo * 8, 8), 8)
            pc_z = pl.ds(pl.multiple_of(T + zo * 8, 8), 8)
            pc_q = pl.ds(pl.multiple_of(S + zo * 16, 16), 16)

            def pieces(kind):
                LB = 16
                if kind == "lnx":
                    def f(u, val):
                        q_v[pc_q, 0:128] = val.astype(bf16)
                        rc = pl.ds(pl.multiple_of(tn * T + u * LB, LB), LB)
                        st(xn2_s, u * LB, _ln(q_v[rc, :].astype(f32)).astype(bf16))
                    return [(f, u) for u in range(T // LB)]
                if kind == "lnz":
                    def f(u, val):
                        z2f_s[pc_z, 0:128] = val[0:8]
                        rc = pl.ds(pl.multiple_of(t * T + u * LB, LB), LB)
                        st(z2_s, t * T + u * LB, _ln(z2f_s[u * LB:(u + 1) * LB, :]).astype(bf16))
                    return [(f, u) for u in range(T // LB)]
                RBp = O["RBp"]

                def f(u, val):
                    kpad_s[pc_k, 0:128] = val[0:8]
                    o = HALO + u * RBp
                    ksh = kpad_s[o:o + RBp, :] * shift_s[0:1, :]
                    for j in range(1, KS):
                        ksh = ksh + kpad_s[o - j:o - j + RBp, :] * shift_s[j:j + 1, :]
                    rc = pl.ds(pl.multiple_of(t * T + u * RBp, RBp), RBp)
                    st(kv_s, t * T + (o - HALO), (ksh * v_v[rc, :].astype(f32)).astype(bf16))
                return [(f, u) for u in range(T // RBp)]

            def zpaced(c0, c1, kind):
                wk = pieces(kind)
                NR = O["NR"]
                acc = None
                wi = 0
                for kt in range(D // 128):
                    ks_ = slice(kt * 128, (kt + 1) * 128)
                    p_ = jnp.dot(ld(xn_s, t * T, T, ks_), win_v[ks_, c0:c1], preferred_element_type=f32)
                    acc = p_ if acc is None else acc + p_
                    hi = min(len(wk), -(-len(wk) * (kt + 1) // NR))
                    n = hi - wi
                    for q_, (f, u) in enumerate(wk[wi:hi]):
                        row = (q_ * T // n) // 16 * 16
                        f(u, p_[row:row + 16, 0:128])
                    wi = hi
                for cc in range(c0, c1, 128):
                    gz = gelu(acc[:, cc - c0:cc - c0 + 128])
                    if cc >= FH:
                        z2f_s[0:T, cc - FH:cc - FH + 128] = gz
                    else:
                        st(z1_s, t * T, gz.astype(bf16), slice(cc, cc + 128))

            def halo():
                kpad_s[0:HALO, :] = kpad_s[T:T + HALO, :]

            fns = dict(K=kdft, P=kpad, V=kv_chunk, X=xdft, Z=zdot, Y=zpaced)
            waits = dict(q0=lambda: q_copy(0).wait(), ssm=cs.wait,
                         kv=lambda: (ck.wait(), cv.wait()),
                         q1=lambda: q_copy(tn).wait(),
                         w0=lambda: win_copy(0).wait(), w1=lambda: win_copy(1).wait(),
                         w2=lambda: win_copy(2).wait())

            def body(order):
                for item in order:
                    if item == "lnx":
                        lnx()
                    elif item == "lnz":
                        lnz()
                    elif item == "halo":
                        halo()
                    elif item == "ln0":
                        ln0()
                    elif item == "prefetch":
                        prefetch()
                    elif item in waits:
                        waits[item]()
                    else:
                        fns[item[0]](*item[1:])
                xn_s[hrows(tn * T, T), :] = xn2_s[...]

            @pl.when(t == 0)
            def _():
                body(O["order0"])

            @pl.when(t > 0)
            def _():
                prefetch()
                cs.wait()
                ck.wait()
                cv.wait()

                @pl.when(t + 1 < NT)
                def _():
                    q_copy(t + 1).wait()

                body(O["order"])

        @pl.when(jnp.logical_and(step >= NT, step < 2 * NT))
        @jax.named_scope('phC1')
        def _():
            t = step - NT
            r = rows(t)
            for c in wsp_copy(t):
                c.wait()
            b = bsp_ref[r].astype(f32).reshape(1, T)
            bcol = jnp.transpose(jnp.broadcast_to(b, (128, T)))

            terms = [(fb, lt, i, j) for fb in range(FB // 8) for lt in range(D // 128)
                     for i in _OPT['iorder'] for j in range(i + 1)]
            G = _OPT['G']
            work = [terms[u:u + G] for u in range(0, len(terms), G)]
            acc_c = [None, None]

            def mac(piece):
                for fb, lt, i, j in piece:
                    f0 = pl.multiple_of(t * FB + fb * 8, 8)
                    fre = pl.ds(f0, 8)
                    fim = pl.ds(f0 + IM, 8)
                    ls = slice(lt * 128, (lt + 1) * 128)
                    xr = xf_s[j, fre, ls]
                    xi = xf_s[j, fim, ls]
                    kr = kf_s[i - j, fre, ls]
                    ki = kf_s[i - j, fim, ls]
                    if j == 0:
                        are = xr * kr - xi * ki
                        aim = xr * ki + xi * kr
                    else:
                        are = acc_c[0] + xr * kr - xi * ki
                        aim = acc_c[1] + xr * ki + xi * kr
                    acc_c[0], acc_c[1] = are, aim
                    if j == i:
                        sf_s[i, fre, ls] = are
                        sf_s[i, fim, ls] = aim

            pace = pl.ds(pl.multiple_of(zero_s[0] * 8, 8), 8)
            KQ = _OPT['KQ']
            rh = pl.ds(pl.multiple_of(t * (T // 2), T // 2), T // 2)
            nround = (FH // 128) * KQ
            wi = 0
            for c in range(FH // 128):
                cs_ = slice(c * 128, (c + 1) * 128)
                acc = None
                for kq in range(KQ):
                    ks_ = slice(kq * (S // KQ), (kq + 1) * (S // KQ))
                    nk = S // 128 // KQ
                    lhs = jnp.concatenate([pltpu.bitcast(wsp_v[k, rh, :], bf16) for k in range(kq * nk, (kq + 1) * nk)], axis=1)
                    p = jnp.dot(lhs, ld(z2_s, kq * (S // KQ), S // KQ, cs_), preferred_element_type=f32)
                    acc = p if acc is None else acc + p
                    rd = c * KQ + kq
                    hi = -(-len(work) * (rd + 1) // nround)
                    n = hi - wi
                    for q_, w in enumerate(work[wi:hi]):
                        row = (q_ * T // n) // 8 * 8
                        xf_s[NC, pace, 0:128] = p[row:row + 8, :]
                        mac(w)
                    wi = hi
                h = ld(z1_s, t * T, T, cs_).astype(f32) * (acc + bcol)
                st(z1_s, t * T, h.astype(bf16), cs_)

        @pl.when(step >= 2 * NT)
        @jax.named_scope('phC2')
        def _():
            t = step - 2 * NT
            r = rows(t)

            @pl.when(t == 0)
            def _():
                wout_copy().wait()

            o = jnp.dot(ld(z1_s, t * T, T), wout_v[...], preferred_element_type=f32)
            ho = 0.5 * o
            gate = ho + ho * jnp.tanh(ho)
            inv = inv_ref[...]
            dvec = dvec_ref[...].astype(f32).reshape(1, D)
            H = _C // 2
            for c in range(CPT):
                i = t * CPT + c
                cur = jnp.concatenate([sf_s[i, 0:_C, :], sf_s[i, IM:IM + _C, :]], axis=0)
                ip = jnp.maximum(i - 1, 0)
                pre, pim = sf_s[ip, 0:_C, :], sf_s[ip, IM:IM + _C, :]
                if c == 0:
                    pre = jnp.where(t > 0, pre, 0.0)
                    pim = jnp.where(t > 0, pim, 0.0)
                add = jnp.concatenate(
                    [-pim[:H], pim[H:], pre[:H], -pre[H:]], axis=0)
                tt = (cur + add).astype(bf16)
                y = jnp.dot(inv, tt, preferred_element_type=f32)
                rc = pl.ds(pl.multiple_of(t * T + c * _C, _C), _C)
                y = y + ld(kv_s, t * T + c * _C, _C).astype(f32) * dvec
                s = ld(xn_s, t * T + c * _C, _C).astype(f32) * y
                out = q_v[rc, :].astype(f32) + s * gate[c * _C:(c + 1) * _C, :]
                o_ref[c * _C:(c + 1) * _C, :] = out.astype(o_ref.dtype)

    full = lambda shape: pl.BlockSpec(shape, lambda s: (0,) * len(shape))
    anyspec = pl.BlockSpec(memory_space=pl.ANY)
    out = pl.pallas_call(
        kernel,
        grid=(3 * NT,),
        in_specs=[anyspec] * 7 + [
            full((KS, D)), full((D,)), full((S,)),
            full((2 * _C, _C)), full((_C, 2 * _C)),
        ],
        out_specs=pl.BlockSpec((None, T, D),
                               lambda s: (0, jnp.maximum(s - 2 * NT, 0), 0)),
        out_shape=jax.ShapeDtypeStruct((1, S, D), A_q.dtype),
        scratch_shapes=[
            pltpu.VMEM((S + 32, D), bf16), pltpu.VMEM((S, D), bf16),
            pltpu.VMEM((S, D), bf16), pltpu.VMEM((D, S), bf16),
            pltpu.VMEM((D, F2), bf16), pltpu.VMEM((S // 128, S // 2, 128), jnp.uint32),
            pltpu.VMEM((FH, D), bf16),
            pltpu.VMEM((S // 2, D), jnp.uint32), pltpu.VMEM((S // 2, D), jnp.uint32),
            pltpu.VMEM((S // 2, FH), jnp.uint32), pltpu.VMEM((S // 2, FH), jnp.uint32),
            pltpu.VMEM((NC + 1, IM + _C, D), f32), pltpu.VMEM((NC, IM + _C, D), f32),
            pltpu.VMEM((NC, IM + _C, D), f32),
            pltpu.VMEM((T + HALO + 16, D), f32), pltpu.VMEM((8, D), f32),
            pltpu.VMEM((T + 16, FH), f32), pltpu.VMEM((T // 2, D), jnp.uint32),
            pltpu.SMEM((1,), jnp.int32),
            pltpu.SemaphoreType.DMA((7, NT)),
        ],
        compiler_params=pltpu.CompilerParams(
            dimension_semantics=("arbitrary",),
            vmem_limit_bytes=110 * 1024 * 1024,
        ),
    )(A_q, A_k, A_v, A_ssm_k, B_w_in, B_w_sp, B_w_out,
      A_shift_k.T, A_ssm_D, B_b_sp,
      jnp.asarray(_FWD, bf16), jnp.asarray(_INV, bf16))
    return out
```

```python
import numpy as np
import jax
import jax.numpy as jnp
import jax.experimental.pallas as pl
import jax.experimental.pallas.tpu as pltpu

_C = 128


def _dft_mats():
    n = np.arange(_C)
    f = np.concatenate([np.arange(0, _C, 2), np.arange(1, _C, 2)])
    th = 2.0 * np.pi * (f[:, None] + 0.5) * n[None, :] / (2 * _C)
    fwd = np.concatenate([np.cos(th), -np.sin(th)], axis=0)
    inv = np.concatenate([np.cos(th).T, -np.sin(th).T], axis=1) / _C
    return fwd.astype(np.float32), inv.astype(np.float32)


_FWD, _INV = _dft_mats()
_OPT = dict(NR=4, RBp=32, G=5, iorder=list(range(16)), pad=8, late_gelu=False, KQ=4, groups=[[i] for i in range(16)], RB=32, LB=16, MB=512, order=[
    ("K", 0), ("K", 1), ("K", 2), ("K", 3), ("P", 0), ("P", 1), ("P", 2), ("P", 3),
    ("Z", 1024, 1536), ("V", 0), ("X", 0), ("V", 1), ("X", 1), "lnx",
    ("Z", 512, 1024), ("V", 2), ("X", 2), ("V", 3), ("X", 3), "halo",
    ("Z", 0, 512), "lnz"],
    order0=["q0", "ln0", "w2", ("Z", 1024, 1536), "ssm", ("K", 0), ("K", 1), ("K", 2), ("K", 3),
            "w1", ("Z", 512, 1024), "kv", ("P", 0), ("P", 1), ("P", 2), ("P", 3), "prefetch",
            ("V", 0), ("X", 0), ("V", 1), ("X", 1), ("V", 2), ("X", 2), ("V", 3), ("X", 3), "halo",
            "w0", "q1", ("Z", 0, 512), "lnz", "lnx"])


_G1 = float(np.sqrt(2.0 / np.pi))
_G2 = float(np.sqrt(2.0 / np.pi) * 0.044715)


def _gelu(x):
    h = 0.5 * x
    return h + h * jnp.tanh(x * (_G1 + _G2 * (x * x)))


def _ln(x):
    m = jnp.mean(x, axis=-1, keepdims=True)
    xc = x - m
    v = jnp.mean(xc * xc, axis=-1, keepdims=True)
    return xc * jax.lax.rsqrt(v + 1e-5)


def pallas_recurrent_scan__ssm_conv_h3__mixer_gmlp__prompt_kernel(
    A_q: jax.Array,
    A_k: jax.Array,
    A_v: jax.Array,
    A_shift_k: jax.Array,
    A_ssm_k: jax.Array,
    A_ssm_D: jax.Array,
    B_x: jax.Array,
    B_w_in: jax.Array,
    B_w_sp: jax.Array,
    B_b_sp: jax.Array,
    B_w_out: jax.Array,
):
    del B_x
    _, S, D = A_q.shape
    KS = A_shift_k.shape[-1]
    F2 = B_w_in.shape[-1]
    FH = F2 // 2
    T = 512
    NT = S // T
    CPT = T // _C
    NC = S // _C
    FB = _C // NT
    HALO = 8
    IM = _C + _OPT['pad']
    NW_COLS = 128
    bf16, f32 = jnp.bfloat16, jnp.float32

    def kernel(q_h, k_h, v_h, ssm_h, win_h, wsp_h, wout_h,
               shift_ref, dvec_ref, bsp_ref, fwd_ref, inv_ref,
               o_ref,
               q_v, k_v, v_v, ssm_v, win_v, wsp_v, wout_v,
               xn_s, kv_s, z1_s, z2_s, xf_s, kf_s, sf_s, kpad_s, shift_s, z2f_s, xn2_s, zero_s,
               sems):
        step = pl.program_id(0)

        def rows(t):
            return pl.ds(pl.multiple_of(t * T, T), T)

        def hrows(r0, n):
            if isinstance(r0, int):
                return slice(r0 // 2, (r0 + n) // 2)
            return pl.ds(pl.multiple_of(r0 // 2, n // 2), n // 2)

        def st(ref, r0, val, cs=slice(None)):
            ref[hrows(r0, val.shape[0]), cs] = pltpu.bitcast(val, jnp.uint32)

        def ld(ref, r0, n, cs=slice(None)):
            return pltpu.bitcast(ref[hrows(r0, n), cs], bf16)

        def q_copy(t):
            r = rows(t)
            return pltpu.make_async_copy(q_h.at[0, r, :], q_v.at[r, :], sems.at[0, t])

        def tile_copies(t):
            r = rows(t)
            return (
                pltpu.make_async_copy(k_h.at[0, r, :], k_v.at[r, :], sems.at[1, t]),
                pltpu.make_async_copy(v_h.at[0, r, :], v_v.at[r, :], sems.at[2, t]),
                pltpu.make_async_copy(ssm_h.at[:, r], ssm_v.at[:, r], sems.at[3, t]),
            )

        def wsp_copy(t):
            r = rows(t)
            return [pltpu.make_async_copy(wsp_h.at[r, k * 128:(k + 1) * 128], wsp_v.bitcast(bf16).at[k, r, :],
                                          sems.at[4, t]) for k in range(S // 128)]

        def win_copy(c):
            cs_ = pl.ds(c * 512, 512)
            return pltpu.make_async_copy(win_h.at[:, cs_], win_v.at[:, cs_], sems.at[6, c])

        def wout_copy():
            return pltpu.make_async_copy(wout_h, wout_v, sems.at[5, 1])

        @pl.when(step == 0)
        def _():
            ck, cv, cs = tile_copies(0)
            q_copy(0).start()
            win_copy(2).start()
            cs.start()
            win_copy(1).start()
            ck.start()
            cv.start()
            win_copy(0).start()
            q_copy(1).start()
            kpad_s[0:HALO, :] = jnp.zeros((HALO, D), f32)
            zero_s[0] = 0
            shift_s[0:KS, :] = shift_ref[...].astype(f32)

        @pl.when(step < NT)
        @jax.named_scope('phB')
        def _():
            t = step

            tn = jnp.minimum(t + 1, NT - 1)

            def prefetch():
                @pl.when(t + 1 < NT)
                def _():
                    for c in tile_copies(t + 1):
                        c.start()

                @pl.when(t + 2 < NT)
                def _():
                    q_copy(t + 2).start()

                for c in wsp_copy(t):
                    c.start()

                @pl.when(t == 1)
                def _():
                    wout_copy().start()

            r = rows(t)
            ck, cv, cs = tile_copies(t)

            def ln0():
                for c in range(T // 16):
                    rc = slice(c * 16, (c + 1) * 16)
                    st(xn_s, c * 16, _ln(q_v[rc, :].astype(f32)).astype(bf16))

            fwd = fwd_ref[...]
            O = _OPT

            def kdft(c):
                blk = ssm_v[:, pl.ds(pl.multiple_of(t * T + c * _C, _C), _C)]
                res = jax.lax.dot_general(
                    fwd, blk, (((1,), (1,)), ((), ())), preferred_element_type=f32)
                kf_s[t * CPT + c, 0:_C, :] = res[:_C]
                kf_s[t * CPT + c, IM:IM + _C, :] = res[_C:]

            def gelu(z):
                return _gelu(z)

            RB = O["RB"]

            def kpad(c):
                rc = pl.ds(pl.multiple_of(t * T + c * _C, _C), _C)
                kpad_s[HALO + c * _C:HALO + (c + 1) * _C, :] = k_v[rc, :].astype(f32)

            def kv_chunk(c):
                for u in range(_C // RB):
                    o = HALO + c * _C + u * RB
                    ksh = kpad_s[o:o + RB, :] * shift_s[0:1, :]
                    for j in range(1, KS):
                        ksh = ksh + kpad_s[o - j:o - j + RB, :] * shift_s[j:j + 1, :]
                    rc = pl.ds(pl.multiple_of(t * T + c * _C + u * RB, RB), RB)
                    st(kv_s, t * T + (o - HALO), (ksh * v_v[rc, :].astype(f32)).astype(bf16))

            def xdft(c):
                rc = pl.ds(pl.multiple_of(t * T + c * _C, _C), _C)
                res = jnp.dot(fwd, ld(kv_s, t * T + c * _C, _C), preferred_element_type=f32)
                xf_s[t * CPT + c, 0:_C, :] = res[:_C]
                xf_s[t * CPT + c, IM:IM + _C, :] = res[_C:]

            def lnx(h=None):
                LB = O["LB"]
                n_ = T // LB
                for u in (range(n_) if h is None else range(h * n_ // 2, (h + 1) * n_ // 2)):
                    rc = pl.ds(pl.multiple_of(tn * T + u * LB, LB), LB)
                    st(xn2_s, u * LB, _ln(q_v[rc, :].astype(f32)).astype(bf16))

            def lnz(h=None):
                LB = O["LB"]
                n_ = T // LB
                for u in (range(n_) if h is None else range(h * n_ // 2, (h + 1) * n_ // 2)):
                    rc = pl.ds(pl.multiple_of(t * T + u * LB, LB), LB)
                    st(z2_s, t * T + u * LB, _ln(z2f_s[u * LB:(u + 1) * LB, :]).astype(bf16))

            def zdot(c0, c1, ms=None, MB=None):
                MB = MB or O["MB"]
                for m in (range(T // MB) if ms is None else ms):
                    rm = pl.ds(pl.multiple_of(t * T + m * MB, MB), MB)
                    z = jnp.dot(ld(xn_s, t * T + m * MB, MB), win_v[:, c0:c1], preferred_element_type=f32)
                    for cc in range(c0, c1, 128):
                        gz = z[:, cc - c0:cc - c0 + 128]
                        if cc >= FH or not O["late_gelu"]:
                            gz = gelu(gz)
                        if cc >= FH:
                            z2f_s[m * MB:(m + 1) * MB, cc - FH:cc - FH + 128] = gz
                        else:
                            st(z1_s, t * T + m * MB, gz.astype(bf16), slice(cc, cc + 128))

            zo = zero_s[0]
            pc_k = pl.ds(pl.multiple_of(HALO + T + zo * 8, 8), 8)
            pc_z = pl.ds(pl.multiple_of(T + zo * 8, 8), 8)
            pc_q = pl.ds(pl.multiple_of(S + zo * 16, 16), 16)

            def pieces(kind):
                LB = 16
                if kind == "lnx":
                    def f(u, val):
                        q_v[pc_q, 0:128] = val.astype(bf16)
                        rc = pl.ds(pl.multiple_of(tn * T + u * LB, LB), LB)
                        st(xn2_s, u * LB, _ln(q_v[rc, :].astype(f32)).astype(bf16))
                    return [(f, u) for u in range(T // LB)]
                if kind == "lnz":
                    def f(u, val):
                        z2f_s[pc_z, 0:128] = val[0:8]
                        rc = pl.ds(pl.multiple_of(t * T + u * LB, LB), LB)
                        st(z2_s, t * T + u * LB, _ln(z2f_s[u * LB:(u + 1) * LB, :]).astype(bf16))
                    return [(f, u) for u in range(T // LB)]
                RBp = O["RBp"]

                def f(u, val):
                    kpad_s[pc_k, 0:128] = val[0:8]
                    o = HALO + u * RBp
                    ksh = kpad_s[o:o + RBp, :] * shift_s[0:1, :]
                    for j in range(1, KS):
                        ksh = ksh + kpad_s[o - j:o - j + RBp, :] * shift_s[j:j + 1, :]
                    rc = pl.ds(pl.multiple_of(t * T + u * RBp, RBp), RBp)
                    st(kv_s, t * T + (o - HALO), (ksh * v_v[rc, :].astype(f32)).astype(bf16))
                return [(f, u) for u in range(T // RBp)]

            def zpaced(c0, c1, kind):
                wk = pieces(kind)
                NR = O["NR"]
                acc = None
                wi = 0
                for kt in range(D // 128):
                    ks_ = slice(kt * 128, (kt + 1) * 128)
                    p_ = jnp.dot(ld(xn_s, t * T, T, ks_), win_v[ks_, c0:c1], preferred_element_type=f32)
                    acc = p_ if acc is None else acc + p_
                    hi = min(len(wk), -(-len(wk) * (kt + 1) // NR))
                    n = hi - wi
                    for q_, (f, u) in enumerate(wk[wi:hi]):
                        row = (q_ * T // n) // 16 * 16
                        f(u, p_[row:row + 16, 0:128])
                    wi = hi
                for cc in range(c0, c1, 128):
                    gz = gelu(acc[:, cc - c0:cc - c0 + 128])
                    if cc >= FH:
                        z2f_s[0:T, cc - FH:cc - FH + 128] = gz
                    else:
                        st(z1_s, t * T, gz.astype(bf16), slice(cc, cc + 128))

            def halo():
                kpad_s[0:HALO, :] = kpad_s[T:T + HALO, :]

            fns = dict(K=kdft, P=kpad, V=kv_chunk, X=xdft, Z=zdot, Y=zpaced, LX=lnx, LZ=lnz)
            waits = dict(q0=lambda: q_copy(0).wait(), ssm=cs.wait,
                         kv=lambda: (ck.wait(), cv.wait()),
                         q1=lambda: q_copy(tn).wait(),
                         w0=lambda: win_copy(0).wait(), w1=lambda: win_copy(1).wait(),
                         w2=lambda: win_copy(2).wait())

            def body(order):
                for item in order:
                    if item == "lnx":
                        lnx()
                    elif item == "lnz":
                        lnz()
                    elif item == "halo":
                        halo()
                    elif item == "ln0":
                        ln0()
                    elif item == "prefetch":
                        prefetch()
                    elif item in waits:
                        waits[item]()
                    else:
                        fns[item[0]](*item[1:])
                xn_s[hrows(tn * T, T), :] = xn2_s[...]

            @pl.when(t == 0)
            def _():
                body(O["order0"])

            @pl.when(t > 0)
            def _():
                prefetch()
                cs.wait()
                ck.wait()
                cv.wait()

                @pl.when(t + 1 < NT)
                def _():
                    q_copy(t + 1).wait()

                body(O["order"])

        @pl.when(jnp.logical_and(step >= NT, step < 2 * NT))
        @jax.named_scope('phC1')
        def _():
            t = step - NT
            r = rows(t)
            for c in wsp_copy(t):
                c.wait()
            b = bsp_ref[r].astype(f32).reshape(1, T)
            bcol = jnp.transpose(jnp.broadcast_to(b, (128, T)))

            terms = [(fb, lt, i, j) for fb in range(FB // 8) for lt in range(D // 128)
                     for i in _OPT['iorder'] for j in range(i + 1)]
            G = _OPT['G']
            work = [terms[u:u + G] for u in range(0, len(terms), G)]
            acc_c = [None, None]

            def mac(piece):
                for fb, lt, i, j in piece:
                    f0 = pl.multiple_of(t * FB + fb * 8, 8)
                    fre = pl.ds(f0, 8)
                    fim = pl.ds(f0 + IM, 8)
                    ls = slice(lt * 128, (lt + 1) * 128)
                    xr = xf_s[j, fre, ls]
                    xi = xf_s[j, fim, ls]
                    kr = kf_s[i - j, fre, ls]
                    ki = kf_s[i - j, fim, ls]
                    if j == 0:
                        are = xr * kr - xi * ki
                        aim = xr * ki + xi * kr
                    else:
                        are = acc_c[0] + xr * kr - xi * ki
                        aim = acc_c[1] + xr * ki + xi * kr
                    acc_c[0], acc_c[1] = are, aim
                    if j == i:
                        sf_s[i, fre, ls] = are
                        sf_s[i, fim, ls] = aim

            pace = pl.ds(pl.multiple_of(zero_s[0] * 8, 8), 8)
            KQ = _OPT['KQ']
            rh = pl.ds(pl.multiple_of(t * (T // 2), T // 2), T // 2)
            nround = (FH // 128) * KQ
            wi = 0
            for c in range(FH // 128):
                cs_ = slice(c * 128, (c + 1) * 128)
                acc = None
                for kq in range(KQ):
                    ks_ = slice(kq * (S // KQ), (kq + 1) * (S // KQ))
                    nk = S // 128 // KQ
                    lhs = jnp.concatenate([pltpu.bitcast(wsp_v[k, rh, :], bf16) for k in range(kq * nk, (kq + 1) * nk)], axis=1)
                    p = jnp.dot(lhs, ld(z2_s, kq * (S // KQ), S // KQ, cs_), preferred_element_type=f32)
                    acc = p if acc is None else acc + p
                    rd = c * KQ + kq
                    hi = -(-len(work) * (rd + 1) // nround)
                    n = hi - wi
                    for q_, w in enumerate(work[wi:hi]):
                        row = (q_ * T // n) // 8 * 8
                        xf_s[NC, pace, 0:128] = p[row:row + 8, :]
                        mac(w)
                    wi = hi
                h = ld(z1_s, t * T, T, cs_).astype(f32) * (acc + bcol)
                st(z1_s, t * T, h.astype(bf16), cs_)

        @pl.when(step >= 2 * NT)
        @jax.named_scope('phC2')
        def _():
            t = step - 2 * NT
            r = rows(t)

            @pl.when(t == 0)
            def _():
                wout_copy().wait()

            o = jnp.dot(ld(z1_s, t * T, T), wout_v[...], preferred_element_type=f32)
            ho = 0.5 * o
            gate = ho + ho * jnp.tanh(ho)
            inv = inv_ref[...]
            dvec = dvec_ref[...].astype(f32).reshape(1, D)
            H = _C // 2
            for c in range(CPT):
                i = t * CPT + c
                cur = jnp.concatenate([sf_s[i, 0:_C, :], sf_s[i, IM:IM + _C, :]], axis=0)
                ip = jnp.maximum(i - 1, 0)
                pre, pim = sf_s[ip, 0:_C, :], sf_s[ip, IM:IM + _C, :]
                if c == 0:
                    pre = jnp.where(t > 0, pre, 0.0)
                    pim = jnp.where(t > 0, pim, 0.0)
                add = jnp.concatenate(
                    [-pim[:H], pim[H:], pre[:H], -pre[H:]], axis=0)
                tt = (cur + add).astype(bf16)
                y = jnp.dot(inv, tt, preferred_element_type=f32)
                rc = pl.ds(pl.multiple_of(t * T + c * _C, _C), _C)
                y = y + ld(kv_s, t * T + c * _C, _C).astype(f32) * dvec
                s = ld(xn_s, t * T + c * _C, _C).astype(f32) * y
                out = q_v[rc, :].astype(f32) + s * gate[c * _C:(c + 1) * _C, :]
                o_ref[c * _C:(c + 1) * _C, :] = out.astype(o_ref.dtype)

    full = lambda shape: pl.BlockSpec(shape, lambda s: (0,) * len(shape))
    anyspec = pl.BlockSpec(memory_space=pl.ANY)
    out = pl.pallas_call(
        kernel,
        grid=(3 * NT,),
        in_specs=[anyspec] * 7 + [
            full((KS, D)), full((D,)), full((S,)),
            full((2 * _C, _C)), full((_C, 2 * _C)),
        ],
        out_specs=pl.BlockSpec((None, T, D),
                               lambda s: (0, jnp.maximum(s - 2 * NT, 0), 0)),
        out_shape=jax.ShapeDtypeStruct((1, S, D), A_q.dtype),
        scratch_shapes=[
            pltpu.VMEM((S + 32, D), bf16), pltpu.VMEM((S, D), bf16),
            pltpu.VMEM((S, D), bf16), pltpu.VMEM((D, S), bf16),
            pltpu.VMEM((D, F2), bf16), pltpu.VMEM((S // 128, S // 2, 128), jnp.uint32),
            pltpu.VMEM((FH, D), bf16),
            pltpu.VMEM((S // 2, D), jnp.uint32), pltpu.VMEM((S // 2, D), jnp.uint32),
            pltpu.VMEM((S // 2, FH), jnp.uint32), pltpu.VMEM((S // 2, FH), jnp.uint32),
            pltpu.VMEM((NC + 1, IM + _C, D), f32), pltpu.VMEM((NC, IM + _C, D), f32),
            pltpu.VMEM((NC, IM + _C, D), f32),
            pltpu.VMEM((T + HALO + 16, D), f32), pltpu.VMEM((8, D), f32),
            pltpu.VMEM((T + 16, FH), f32), pltpu.VMEM((T // 2, D), jnp.uint32),
            pltpu.SMEM((1,), jnp.int32),
            pltpu.SemaphoreType.DMA((7, NT)),
        ],
        compiler_params=pltpu.CompilerParams(
            dimension_semantics=("arbitrary",),
            vmem_limit_bytes=110 * 1024 * 1024,
        ),
    )(A_q, A_k, A_v, A_ssm_k, B_w_in, B_w_sp, B_w_out,
      A_shift_k.T, A_ssm_D, B_b_sp,
      jnp.asarray(_FWD, bf16), jnp.asarray(_INV, bf16))
    return out
```
